```python
import os as _os
_os.environ.setdefault("JAX_PLATFORMS", "cpu")
import jax
import jax.numpy as jnp

def _softmax(x, axis=-1):
    return jax.nn.softmax(x, axis=axis)
def _gelu(x):
    return jax.nn.gelu(x, approximate=True)
def _silu(x):
    return jax.nn.silu(x)
def _sigmoid(x):
    return jax.nn.sigmoid(x)
def _layernorm(x, axis=-1, eps=1e-5):
    m = jnp.mean(x, axis=axis, keepdims=True)
    v = jnp.var(x, axis=axis, keepdims=True)
    return (x - m) / jnp.sqrt(v + eps)
def _scatter_add(tgt, idx, src, axis=0):
    return tgt.at[idx].add(src)
def _segment_sum(src, seg, n):
    return jax.ops.segment_sum(src, seg, n)
class _Rng:
    def __init__(self, key):
        self._k = key
    def _next(self):
        self._k, sub = jax.random.split(self._k)
        return sub
    def normal(self, shape):
        return jax.random.normal(self._next(), shape, dtype=jnp.bfloat16)
    def randint(self, lo, hi, shape):
        return jax.random.randint(self._next(), shape, lo, hi, dtype=jnp.int32)
    def uniform(self, shape, lo=0.0, hi=1.0):
        return jax.random.uniform(self._next(), shape, jnp.bfloat16, lo, hi)
    def permutation(self, n):
        return jax.random.permutation(self._next(), n)


kernel_name = 'standalone__geglu_ffn__prompt'

def setup_inputs():
    _rng = _Rng(jax.random.key(int.from_bytes(__import__("os").urandom(4), "little")))
    _w = (lambda a: (lambda t: t.astype(jnp.bfloat16) if jnp.issubdtype(t.dtype, jnp.floating) else t)(jnp.asarray(a)))
    B, S, D, F = 1, 2048, 576, 4608
    return {
        "x": _w((lambda *s: _rng.normal(s) * 0.05)(B, S, D)),
        "w_gate": _w((lambda *s: _rng.normal(s) * 0.05)(D, F)),
        "w_up": _w((lambda *s: _rng.normal(s) * 0.05)(D, F)),
        "w_down": _w((lambda *s: _rng.normal(s) * 0.05)(F, D)),
    }

def reference(x, w_gate, w_up, w_down):
    return (_gelu(x @ w_gate) * (x @ w_up)) @ w_down
```

```python
import jax
import jax.numpy as jnp
from jax import lax
import jax.experimental.pallas as pl
import jax.experimental.pallas.tpu as pltpu

_NT = (((1,), (1,)), ((), ()))
_F32 = jnp.float32
_BF = jnp.bfloat16

_T0 = 512
_TS = 384
_HEAD = (128, 256, 640)
_NL = 4
_XSPLIT = 2
_OG = 128


def _act(g, u):
    return (jax.nn.gelu(g, approximate=True) * u).astype(_BF)


def _mo(v):
    return v if isinstance(v, int) else pl.multiple_of(v, 128)


def _kernel(xT_hbm, wg_hbm, wu_hbm, wd_hbm, o_hbm, buf, x_v, h0_v, acc_v, o_v, sem):
    D, M = o_v.shape
    F = wg_hbm.shape[1]
    t0, ts, head, nl = _T0, _TS, _HEAD, _NL
    nh = len(head)
    hoff = [sum(head[:j]) for j in range(nh + 1)]
    H = hoff[-1]
    lf = (F - H) // nl
    hc = H // nl
    nm = (M - t0) // ts
    xp = t0 // _XSPLIT
    xr = (M - t0) // nl
    srcs = dict(x=(xT_hbm, 0), g=(wg_hbm, M), u=(wu_hbm, M + F), d=(wd_hbm, M + 2 * F))

    def cp(k, off, size, s):
        src, base = srcs[k]
        return pltpu.make_async_copy(src.at[:, pl.ds(_mo(off), size)],
                                     buf.at[:, pl.ds(_mo(base + off), size)], sem.at[s])

    def rd(k, off, size):
        return buf[:, pl.ds(_mo(srcs[k][1] + off), size)]

    def ocp(off, size):
        sl = pl.ds(off, size)
        return pltpu.make_async_copy(o_v.at[:, sl], o_hbm.at[:, sl], sem.at[0])

    def x_cps(p):
        return [cp('x', p * xp, xp, 1 + p)]

    def head_cps(j):
        return [cp(k, hoff[j], head[j], 1 + _XSPLIT + j) for k in 'gu']

    def loop_cps(j):
        s = 1 + _XSPLIT + nh + j
        return ([cp(k, H + j * lf, lf, s) for k in 'gud']
                + [cp('d', j * hc, hc, s), cp('x', t0 + j * xr, xr, s)])

    for p in range(_XSPLIT):
        for c in x_cps(p):
            c.start()
    for j in range(nh):
        for c in head_cps(j):
            c.start()
    for j in range(nl):
        for c in loop_cps(j):
            c.start()

    acc_v[...] = jnp.zeros_like(acc_v)
    for p in range(_XSPLIT):
        for c in x_cps(p):
            c.wait()
        x_v[p * xp:(p + 1) * xp, :] = rd('x', p * xp, xp).T

    for j in range(nh):
        for c in head_cps(j):
            c.wait()
        nsp = 2 if (head[j] // 128) % 2 == 1 else 1
        rp = t0 // nsp
        for p in range(nsp):
            x = x_v[p * rp:(p + 1) * rp, :]
            g = jnp.dot(x, rd('g', hoff[j], head[j]), preferred_element_type=_F32)
            u = jnp.dot(x, rd('u', hoff[j], head[j]), preferred_element_type=_F32)
            h0_v[p * rp:(p + 1) * rp, hoff[j]:hoff[j + 1]] = _act(g, u)

    def ploop(j, carry):
        off = H + j * lf
        off2 = _mo(j * hc)
        xo = _mo(t0 + j * xr)
        for c in loop_cps(j):
            c.wait()
        g = jnp.dot(x_v[0:t0, :], rd('g', off, lf), preferred_element_type=_F32)
        x_v[pl.ds(xo, xr), :] = rd('x', xo, xr).T
        u = jnp.dot(x_v[0:t0, :], rd('u', off, lf), preferred_element_type=_F32)
        h = _act(g, u)
        y = lax.dot_general(rd('d', off2, hc), h0_v[:, pl.ds(off2, hc)], _NT, preferred_element_type=_F32)
        y = y + lax.dot_general(rd('d', off, lf), h, _NT, preferred_element_type=_F32)
        a = acc_v[...] + y
        acc_v[...] = a
        o_v[:, 0:t0] = a.astype(_BF)
        return carry

    lax.fori_loop(0, nl, ploop, 0)
    ocp(0, t0).start()

    def mloop(i, carry):
        r0 = pl.multiple_of(t0 + i * ts, 128)
        x = x_v[pl.ds(r0, ts), :]
        g = jnp.dot(x, rd('g', 0, F), preferred_element_type=_F32)
        u = jnp.dot(x, rd('u', 0, F), preferred_element_type=_F32)
        h = _act(g, u)
        for q in range(ts // _OG):
            y = lax.dot_general(rd('d', 0, F), h[q * _OG:(q + 1) * _OG, :], _NT, preferred_element_type=_F32)
            oq = pl.multiple_of(r0 + q * _OG, 128)
            o_v[:, pl.ds(oq, _OG)] = y.astype(_BF)
            ocp(oq, _OG).start()
        return carry

    lax.fori_loop(0, nm, mloop, 0)
    pltpu.make_async_copy(o_v, o_hbm, sem.at[0]).wait()


@jax.jit
def pallas_standalone__geglu_ffn__prompt_kernel(x, w_gate, w_up, w_down):
    B, S, D = x.shape
    F = w_gate.shape[1]
    M = B * S
    H = sum(_HEAD)
    assert (F - H) % (128 * _NL) == 0 and H % (128 * _NL) == 0
    assert (M - _T0) % _TS == 0 and (M - _T0) % (128 * _NL) == 0
    xT = x.reshape(M, D).T
    wdT = w_down.T
    outT = pl.pallas_call(
        _kernel,
        in_specs=[pl.BlockSpec(memory_space=pl.ANY)] * 4,
        out_specs=pl.BlockSpec(memory_space=pl.ANY),
        out_shape=jax.ShapeDtypeStruct((D, M), x.dtype),
        scratch_shapes=[
            pltpu.VMEM((D, M + 3 * F), _BF),
            pltpu.VMEM((M, D), _BF),
            pltpu.VMEM((_T0, H), _BF),
            pltpu.VMEM((D, _T0), _F32),
            pltpu.VMEM((D, M), _BF),
            pltpu.SemaphoreType.DMA((1 + _XSPLIT + len(_HEAD) + _NL,)),
        ],
        compiler_params=pltpu.CompilerParams(
            vmem_limit_bytes=100 * 1024 * 1024,
            disable_bounds_checks=True,
            disable_semaphore_checks=True,
        ),
    )(xT, w_gate, w_up, wdT)
    return outT.T.reshape(B, S, D)
```

```python
import contextlib
import jax
import jax.numpy as jnp
from jax import lax
import jax.experimental.pallas as pl
import jax.experimental.pallas.tpu as pltpu

NT = (((1,), (1,)), ((), ()))
F32 = jnp.float32
BF = jnp.bfloat16
C0 = 0.7978845608028654
C1 = C0 * 0.044715
KM = 512
KT = 64


def _act(g, uh):
    t = jnp.tanh(g * (C0 + C1 * (g * g)))
    return ((g * uh) * (1.0 + t)).astype(BF)


def _mo(v):
    return v if isinstance(v, int) else pl.multiple_of(v, 128)


def _dot(a, b):
    return jnp.dot(a, b, preferred_element_type=F32)


def make(t0=512, head=(128, 256, 640), nl=4, vmem=110, x0split=2, n2=(30, 24), scopes=False, ogrp=128):
    ts = 256
    nh = len(head)
    hoff = [sum(head[:j]) for j in range(nh + 1)]
    H = hoff[-1]
    scope = (lambda n: jax.named_scope(n)) if scopes else (lambda n: contextlib.nullcontext())

    def kernel(xT_hbm, wg_hbm, wu_hbm, wd_hbm, o_hbm, keep_hbm,
               buf, pg, pu, pd, pd0, x_v, xu_v, h0_v, acc_v, o_v, wt_v, xb, tall, m_v, sem):
        D, M = o_v.shape
        F = wg_hbm.shape[1]
        lf = (F - H) // nl
        hc = H // nl
        nm = (M - t0) // ts
        xp = t0 // x0split
        xr = (M - t0) // nl
        gpi = xr // 128
        srcs = dict(x=(xT_hbm, 0), g=(wg_hbm, M), u=(wu_hbm, M + F), d=(wd_hbm, M + 2 * F))

        def cp(k, off, size, s):
            src, base = srcs[k]
            return pltpu.make_async_copy(src.at[:, pl.ds(_mo(off), size)],
                                         buf.at[:, pl.ds(_mo(base + off), size)], sem.at[s])
        def rd(k, off, size, r0=0, r1=D):
            return buf[r0:r1, pl.ds(_mo(srcs[k][1] + off), size)]
        packed = dict(g=pg, u=pu, d=pd, d0=pd0)
        def rdp(k, off, size):
            w = rd(k[0], off, size)
            packed[k][:, pl.ds(_mo(off), size)] = pltpu.bitcast(w, jnp.uint32)
            return w
        def rdm(k, off, size, r0=0, r1=D):
            return pltpu.bitcast(packed[k][r0 // 2:r1 // 2, off:off + size], BF)
        def ocp(off, size):
            sl = pl.ds(off, size)
            return pltpu.make_async_copy(o_v.at[:, sl], o_hbm.at[:, sl], sem.at[0])
        def x_cps(p):
            return [cp('x', p * xp, xp, 1 + p)]
        def head_cps(j):
            return [cp(k, hoff[j], head[j], 1 + x0split + j) for k in 'gu']
        def loop_cps(j):
            s = 1 + x0split + nh + j
            return ([cp(k, H + j * lf, lf, s) for k in 'gud'] + [cp('d', j * hc, hc, s), cp('x', t0 + j * xr, xr, s)])

        for p in range(x0split):
            for c in x_cps(p): c.start()
        for j in range(nh):
            for c in head_cps(j): c.start()
        for j in range(nl):
            for c in loop_cps(j): c.start()

        acc_v[...] = jnp.zeros_like(acc_v)
        m_v[...] = jnp.zeros_like(m_v)

        def put_x(rows, xt):
            x_v[rows, :] = xt
            xu_v[rows, :] = (xt.astype(F32) * 0.5).astype(BF)

        def build_wt(off, size):
            wt_v[:, pl.ds(_mo(off), size)] = rd('g', off, size, KM, D).astype(F32)
            wt_v[:, pl.ds(_mo(F + off), size)] = rd('u', off, size, KM, D).astype(F32) * 0.5

        for p in range(x0split):
            with scope(f'xwait{p}'):
                for c in x_cps(p): c.wait()
            put_x(slice(p * xp, (p + 1) * xp), rd('x', p * xp, xp).T)

        for j in range(nh):
            with scope(f'hwait{j}'):
                for c in head_cps(j): c.wait()
            nsp = 2 if (head[j] // 128) % 2 == 1 else 1
            rp = t0 // nsp
            wg_c = rdp('g', hoff[j], head[j])
            wu_c = rdp('u', hoff[j], head[j])
            for p in range(nsp):
                rows = slice(p * rp, (p + 1) * rp)
                g = _dot(x_v[rows, :], wg_c)
                u = _dot(xu_v[rows, :], wu_c)
                h0_v[rows, hoff[j]:hoff[j + 1]] = _act(g, u)
            build_wt(hoff[j], head[j])

        def ploop(j, carry):
            off = H + j * lf
            off2 = _mo(j * hc)
            xo = _mo(t0 + j * xr)
            with scope('lwait'):
                for c_ in loop_cps(j): c_.wait()
            never = m_v[0:8, :] > 0
            g = _dot(x_v[0:t0, :], rdp('g', off, lf))
            put_x(pl.ds(xo, xr), rd('x', xo, xr).T)
            u = _dot(xu_v[0:t0, :], rdp('u', off, lf))
            h = _act(g, u)
            for ref, k_, base in ((x_v, 'g', 0), (xu_v, 'u', F)):
                xB = jnp.concatenate([ref[t0 + 96:t0 + 128, KM:], ref[t0 + 224:t0 + 256, KM:]], axis=0)
                tall[0, :, pl.ds(_mo(base + off), lf)] = _dot(xB, rd(k_, off, lf, KM, D))
                tall[0, :, pl.ds(_mo(base + off2), hc)] = _dot(xB, rd(k_, off2, hc, KM, D))
            y = lax.dot_general(rdp('d0', off2, hc), h0_v[:, pl.ds(off2, hc)], NT, preferred_element_type=F32)
            y = y + lax.dot_general(rdp('d', off, lf), h, NT, preferred_element_type=F32)
            a = acc_v[...] + y
            acc_v[...] = a
            o_v[:, 0:t0] = a.astype(BF)
            build_wt(off, lf)
            xtl = jnp.concatenate([x_v[pl.ds(pl.multiple_of(xo + 128 * q + 96, 32), 32), KM:] for q in range(gpi)],
                                  axis=0).astype(F32)
            prev = None
            zero = jnp.zeros((8, 128), F32)
            for k in range(KT):
                col = jnp.broadcast_to(xtl[:, k:k + 1], (32 * gpi, 128))
                for q in range(gpi):
                    for r in range(0, 32, 8):
                        v = col[32 * q + r:32 * q + r + 8]
                        prev = v if prev is None else v + jnp.where(never, prev, zero)
                        xb[j * gpi + q, k, r:r + 8, :] = prev
            return carry
        lax.fori_loop(0, nl, ploop, 0)
        ocp(0, t0).start()

        def mloop(i, gn):
            r0 = pl.multiple_of(t0 + i * ts, 128)
            never2 = m_v[...] > 0
            t_in, t_out = tall.at[i], tall.at[i + 1]
            outs = []
            for ref, k_, base, nn in ((x_v, 'g', 0, n2[0]), (xu_v, 'u', F, n2[1])):
                x = ref[pl.ds(r0, ts), :]
                xt = x[:, KM:]
                c2 = nn * 128
                inits = []
                if c2:
                    ta = _dot(jnp.concatenate([xt[0:96], xt[128:224]], axis=0), rdm(k_, 0, c2, KM, D))
                    inits.append(jnp.concatenate([ta[0:96], t_in[0:32, base:base + c2],
                                                  ta[96:192], t_in[32:64, base:base + c2]], axis=0))
                if c2 < F:
                    ta = _dot(jnp.concatenate([xt[0:112], xt[128:240]], axis=0), rdm(k_, c2, F - c2, KM, D))
                    inits.append(jnp.concatenate([ta[0:112], t_in[16:32, base + c2:base + F],
                                                  ta[112:224], t_in[48:64, base + c2:base + F]], axis=0))
                init = jnp.concatenate(inits, axis=1) if len(inits) > 1 else inits[0]
                outs.append(_dot(x[:, :KM], rdm(k_, 0, F, 0, KM)) + init)
            for q in range(ts // ogrp):
                h = _act(*[o[q * ogrp:(q + 1) * ogrp, :] for o in outs])
                y = lax.dot_general(jnp.concatenate([rdm('d0', 0, H), rdm('d', H, F - H)], axis=1), h, NT, preferred_element_type=F32)
                oq = pl.multiple_of(r0 + q * ogrp, 128)
                o_v[:, pl.ds(oq, ogrp)] = y.astype(BF)
                ocp(oq, ogrp).start()
            prev = None
            for base, nn in ((0, n2[0]), (F, n2[1])):
                for c in range(F // 128):
                    col = base + 128 * c
                    for q in range(2):
                        for rr in ((0, 16) if c < nn else (16,)):
                            acc = None
                            for k in range(KT):
                                p = xb[gn + q, k, rr:rr + 16, :] * wt_v[k:k + 1, col:col + 128]
                                if acc is None:
                                    acc = p if prev is None else jnp.where(never2, prev, p)
                                else:
                                    acc = acc + p
                            t_out[32 * q + rr:32 * q + rr + 16, col:col + 128] = acc
                            prev = acc
            return jnp.minimum(gn + 2, 2 * (nm - 1))
        with scope('mloop'):
            lax.fori_loop(0, nm, mloop, jnp.int32(2))
        keep = pltpu.make_async_copy(tall.at[1, 16:24, 0:128], keep_hbm, sem.at[1])
        keep.start()
        with scope('owait'):
            pltpu.make_async_copy(o_v, o_hbm, sem.at[0]).wait()
        keep.wait()

    @jax.jit
    def fn(x, w_gate, w_up, w_down):
        B, S, D = x.shape
        F = w_gate.shape[1]
        M = B * S
        assert (F - H) % (128 * nl) == 0 and H % (128 * nl) == 0 and (M - t0) % ts == 0 and (M - t0) % (128 * nl) == 0
        xT = x.reshape(M, D).T
        wdT = w_down.T
        outT, _ = pl.pallas_call(
            kernel,
            in_specs=[pl.BlockSpec(memory_space=pl.ANY)] * 4,
            out_specs=[pl.BlockSpec(memory_space=pl.ANY)] * 2,
            out_shape=[jax.ShapeDtypeStruct((D, M), x.dtype), jax.ShapeDtypeStruct((8, 128), F32)],
            scratch_shapes=[
                pltpu.VMEM((D, M + 3 * F), BF), pltpu.VMEM((D // 2, F), jnp.uint32), pltpu.VMEM((D // 2, F), jnp.uint32), pltpu.VMEM((D // 2, F), jnp.uint32), pltpu.VMEM((D // 2, H), jnp.uint32), pltpu.VMEM((M, D), BF), pltpu.VMEM((M, D), BF),
                pltpu.VMEM((t0, H), BF), pltpu.VMEM((D, t0), F32), pltpu.VMEM((D, M), BF),
                pltpu.VMEM((KT, 2 * F), F32), pltpu.VMEM(((M - t0) // 128, KT, 32, 128), F32),
                pltpu.VMEM(((M - t0) // ts + 1, 64, 2 * F), F32), pltpu.VMEM((16, 128), F32),
                pltpu.SemaphoreType.DMA((1 + x0split + nh + nl,)),
            ],
            compiler_params=pltpu.CompilerParams(vmem_limit_bytes=vmem * 1024 * 1024,
                                                 disable_bounds_checks=True, disable_semaphore_checks=True),
        )(xT, w_gate, w_up, wdT)
        return outT.T.reshape(B, S, D)
    return fn

pallas_standalone__geglu_ffn__prompt_kernel = make()
```

```python
import jax
import jax.numpy as jnp
from jax import lax
import jax.experimental.pallas as pl
import jax.experimental.pallas.tpu as pltpu

_NT = (((1,), (1,)), ((), ()))
_F32 = jnp.float32
_BF = jnp.bfloat16
_U32 = jnp.uint32
_C0 = 0.7978845608028654
_C1 = _C0 * 0.044715

_KM = 512
_KT = 64
_T0 = 512
_TS = 256
_HEAD = (128, 256, 640)
_NL = 4
_XSPLIT = 2
_SLOTW = 4096
_N2 = (32, 32)
_GC = 4
_TREE = (2, 8, 90)
_DSPLIT = (0, 448, 576)


def _act(g, uh):
    t = jnp.tanh(g * (_C0 + _C1 * (g * g)))
    return ((g * (1.0 + t)) * uh).astype(_BF)


def _half(x):
    return (x.astype(_F32) * 0.5).astype(_BF)


def _mo(v):
    return v if isinstance(v, int) else pl.multiple_of(v, 128)


def _dot(a, b):
    return jnp.dot(a, b, preferred_element_type=_F32)


def _dot_nt(a, b):
    return lax.dot_general(a, b, _NT, preferred_element_type=_F32)


def _cat(parts, axis):
    return parts[0] if len(parts) == 1 else jnp.concatenate(parts, axis=axis)


def _kernel(xT_hbm, wg_hbm, wu_hbm, wd_hbm, o_hbm, keep_hbm,
            buf, pg, pu, pd, pd0, x0_v, xu0_v, x_v, xu_v, h0_v, acc_v, o_v,
            wt_v, wts, xb, xb0, tall, m_v, z_s, sem):
    D, M = o_v.shape
    F = wg_hbm.shape[1]
    t0, ts, head, nl = _T0, _TS, _HEAD, _NL
    nh = len(head)
    hoff = [sum(head[:j]) for j in range(nh + 1)]
    H = hoff[-1]
    lf = (F - H) // nl
    hc = H // nl
    nm = (M - t0) // ts
    xp = t0 // _XSPLIT
    xr = (M - t0) // nl
    gpi = xr // 128
    hbm = dict(x=xT_hbm, g=wg_hbm, u=wu_hbm, d=wd_hbm)
    pos0 = dict(x=0, g=t0, u=t0 + H, xs=t0 + 2 * H)
    posl = dict(g=0, u=lf, d=2 * lf, d0=3 * lf, x=3 * lf + hc)

    def cp(k, off, size, slot, pos, s):
        return pltpu.make_async_copy(hbm[k].at[:, pl.ds(_mo(off), size)],
                                     buf.at[slot, :, pos:pos + size], sem.at[s])

    def x_cps(p):
        return [cp('x', p * xp, xp, 0, p * xp, 1 + p)]

    def head_cps(j):
        s = 1 + _XSPLIT + j
        cps = [cp(k, hoff[j], head[j], 0, pos0[k] + hoff[j], s) for k in 'gu']
        if j == nh - 1:
            cps.append(pltpu.make_async_copy(xT_hbm.at[_KM:D, t0:t0 + ts],
                                             buf.at[0, 0:_KT, pos0['xs']:pos0['xs'] + ts], sem.at[s]))
        return cps

    def loop_cps(j):
        s = 1 + _XSPLIT + nh + j
        return ([cp(k, H + j * lf, lf, 1 + j, posl[k], s) for k in 'gud']
                + [cp('d', j * hc, hc, 1 + j, posl['d0'], s),
                   cp('x', t0 + j * xr, xr, 1 + j, posl['x'], s)])

    def rd0(k, off, size, r0=0, r1=D):
        return buf[0, r0:r1, pos0[k] + off:pos0[k] + off + size]

    def rdl(k, j, size, r0=0, r1=D):
        return buf[1 + j, r0:r1, posl[k]:posl[k] + size]

    def keep_packed(ref, slot, off, w):
        ref[slot, :, off:off + w.shape[1]] = pltpu.bitcast(w, _U32)
        return w

    def rdm(k, c0, c1, r0=0, r1=D):
        if k == 'd':
            segs = [(pd0, s, s * hc, hc) for s in range(nl)] + [(pd, s, H + s * lf, lf) for s in range(nl)]
        else:
            ref = pg if k == 'g' else pu
            segs = [(ref, 0, 0, H)] + [(ref, 1 + s, H + s * lf, lf) for s in range(nl)]
        parts = []
        for ref, slot, st, n in segs:
            a, b = max(c0, st), min(c1, st + n)
            if a < b:
                parts.append(ref[slot, r0 // 2:r1 // 2, a - st:b - st])
        return pltpu.bitcast(_cat(parts, 1), _BF)

    for p in range(_XSPLIT):
        for c in x_cps(p):
            c.start()
    for j in range(nh):
        for c in head_cps(j):
            c.start()
    for j in range(nl):
        for c in loop_cps(j):
            c.start()

    acc_v[...] = jnp.zeros_like(acc_v)
    m_v[...] = jnp.zeros_like(m_v)
    for j in range(nl):
        z_s[j] = 0

    def build_xb(xtl, ngrp, dst, g0):
        never = m_v[0:8, :] > 0
        zero = jnp.zeros((8, 128), _F32)
        prev = None
        for k in range(_KT):
            col = jnp.broadcast_to(xtl[:, k:k + 1], (32 * ngrp, 128))
            for q in range(ngrp):
                for r in range(0, 32, 8):
                    v = col[32 * q + r:32 * q + r + 8]
                    prev = v if prev is None else v + jnp.where(never, prev, zero)
                    dst[g0 + q, k, r:r + 8, :] = prev

    def tail_chain(xsrc, g0, cols, dst, prev=None, tsch=(0, 0, 0)):
        never = m_v[...] > 0
        left = sum(2 * len(c[3]) for c in cols)
        for wref, wc, col, units in cols:
            cs = pl.ds(_mo(col), 128)
            for q in range(2):
                for rr in units:
                    tree = tsch[1] if left <= tsch[2] else tsch[0]
                    left -= 1

                    def prod(k):
                        return xsrc[g0 + q, k, rr:rr + 16, :] * wref[pl.ds(k, 1), wc:wc + 128]

                    acc = prod(0) if prev is None else jnp.where(never, prev, prod(0))
                    if tree == 0:
                        acc = lax.fori_loop(1, _KT, lambda k, a: a + prod(k), acc, unroll=True)
                    else:
                        gs = _KT // tree

                        def rest(k0, a):
                            pa = prod(k0 + 1)
                            a = a + (pa + prod(k0 + 2))
                            return lax.fori_loop(3, gs, lambda d, b: b + prod(k0 + d), a, unroll=True)

                        acc = rest(0, acc)
                        acc = lax.fori_loop(1, tree, lambda n, a: rest(n * gs, a + prod(n * gs)), acc,
                                            unroll=True)
                    dst[32 * q + rr:32 * q + rr + 16, cs] = acc
                    prev = acc
        return prev

    for p in range(_XSPLIT):
        for c in x_cps(p):
            c.wait()
        xt = rd0('x', p * xp, xp).T
        x0_v[p * xp:(p + 1) * xp, :] = xt
        xu0_v[p * xp:(p + 1) * xp, :] = _half(xt)

    for j in range(nh):
        for c in head_cps(j):
            c.wait()
        nsp = 2 if (head[j] // 128) % 2 == 1 else 1
        rp = t0 // nsp
        wg_c = keep_packed(pg, 0, hoff[j], rd0('g', hoff[j], head[j]))
        wu_c = keep_packed(pu, 0, hoff[j], rd0('u', hoff[j], head[j]))
        for p in range(nsp):
            rows = slice(p * rp, (p + 1) * rp)
            g = _dot(x0_v[rows, :], wg_c)
            u = _dot(xu0_v[rows, :], wu_c)
            for c in range(hoff[j], hoff[j + 1], 128):
                cl = c - hoff[j]
                h0_v[c // hc, rows, c % hc:c % hc + 128] = _act(g[:, cl:cl + 128], u[:, cl:cl + 128])
        wt_v[0, :, hoff[j]:hoff[j + 1]] = rd0('g', hoff[j], head[j], _KM, D).astype(_F32)
        wt_v[0, :, H + hoff[j]:H + hoff[j + 1]] = rd0('u', hoff[j], head[j], _KM, D).astype(_F32) * 0.5
        if j == nh - 1:
            xs = rd0('xs', 0, ts, 0, _KT).astype(_F32).T
            xs = jnp.concatenate([xs[96:128], xs[224:256]], axis=0)
            tall[0, :, 0:H] = _dot(xs.astype(_BF), rd0('g', 0, H, _KM, D))
            tall[0, :, F:F + H] = _dot((xs * 0.5).astype(_BF), rd0('u', 0, H, _KM, D))
            build_xb(xs, 2, xb0, 0)

    def ploop(j, jc):
        g = _dot(x0_v[...], keep_packed(pg, 1 + j, 0, rdl('g', j, lf)))
        u = _dot(xu0_v[...], keep_packed(pu, 1 + j, 0, rdl('u', j, lf)))
        h = _act(g, u)
        y = _dot_nt(keep_packed(pd0, j, 0, rdl('d0', j, hc)), h0_v[j])
        y = y + _dot_nt(keep_packed(pd, j, 0, rdl('d', j, lf)), h)
        a = acc_v[...] + y
        acc_v[...] = a
        o_v[:, 0:t0] = a.astype(_BF)
        tg = rdl('g', jc, lf, _KM, D).astype(_F32)
        tu = rdl('u', jc, lf, _KM, D).astype(_F32) * 0.5
        wt_v[1 + jc, :, 0:lf] = tg
        wt_v[1 + jc, :, H:H + lf] = tu
        xin = rdl('x', jc, xr)
        wts[:, 0:lf] = tg
        wts[:, lf:2 * lf] = tu
        cols = [(wts, b * lf + c, b * F + H + jc * lf + c, (0, 16)) for b in range(2) for c in range(0, lf, 128)]
        gate = wts[pl.ds(pl.multiple_of(z_s[jc], 8), 16), 0:128]
        last = tail_chain(xb0, 0, cols, tall.at[0], gate)
        mk = jnp.concatenate([m_v[...] > 0] * gpi, axis=1)
        lb = jnp.concatenate([last.astype(_BF)] * gpi, axis=1)
        parts = []
        for r in range(0, D, 128):
            parts.append(jnp.where(mk, lb, xin[r:r + 16]))
            parts.append(xin[r + 16:min(r + 128, D)])
        xt = jnp.concatenate(parts, axis=0).T
        for q in range(gpi):
            x_v[jc * gpi + q] = pltpu.bitcast(xt[128 * q:128 * q + 128], _U32)
            xu_v[jc * gpi + q] = pltpu.bitcast(_half(xt[128 * q:128 * q + 128]), _U32)
        xtl = jnp.concatenate([x_v[jc * gpi + q, 48:64, _KM:] for q in range(gpi)], axis=0)
        build_xb(pltpu.bitcast(xtl, _BF).astype(_F32), gpi, xb, jc * gpi)

        @pl.when(j + 1 < nl)
        def _():
            for c in loop_cps(j + 1):
                c.wait()

        return jnp.minimum(jc + 1, nl - 1)

    for c in loop_cps(0):
        c.wait()
    lax.fori_loop(0, nl, ploop, jnp.int32(0))
    pltpu.make_async_copy(o_v.at[:, 0:t0], o_hbm.at[:, 0:t0], sem.at[0]).start()

    def mloop(i, gn):
        r0 = pl.multiple_of(i * ts, 128)
        t_in, t_out = tall.at[i], tall.at[i + 1]

        def proj(ref, k, base, nn, ca, cb):
            xa, xc = ref[2 * i], ref[2 * i + 1]

            def rows(n, c0, c1):
                return pltpu.bitcast(jnp.concatenate([xa[0:n // 2, c0:c1], xc[0:n // 2, c0:c1]], axis=0), _BF)

            c2 = min(max(nn * 128, ca), cb)
            inits = []
            if c2 > ca:
                ta = _dot(rows(96, _KM, D), rdm(k, ca, c2, _KM, D))
                inits.append(jnp.concatenate([ta[0:96], t_in[0:32, base + ca:base + c2],
                                              ta[96:192], t_in[32:64, base + ca:base + c2]], axis=0))
            if c2 < cb:
                ta = _dot(rows(112, _KM, D), rdm(k, c2, cb, _KM, D))
                inits.append(jnp.concatenate([ta[0:112], t_in[16:32, base + c2:base + cb],
                                              ta[112:224], t_in[48:64, base + c2:base + cb]], axis=0))
            return _dot(rows(128, 0, _KM), rdm(k, ca, cb, 0, _KM)) + _cat(inits, 1)

        hs = [[], []]
        for ca in range(0, F, _GC * 128):
            cb = min(ca + _GC * 128, F)
            g = proj(x_v, 'g', 0, _N2[0], ca, cb)
            u = proj(xu_v, 'u', F, _N2[1], ca, cb)
            for q in range(2):
                hs[q].append(_act(g[q * 128:(q + 1) * 128], u[q * 128:(q + 1) * 128]))
        for q in range(2):
            h = _cat(hs[q], 1)
            oq = pl.ds(pl.multiple_of(t0 + r0 + q * 128, 128), 128)
            cuts = _DSPLIT if q == 1 else (0, D)
            for a, b in zip(cuts[:-1], cuts[1:]):
                o_v[a:b, oq] = _dot_nt(rdm('d', 0, F, a, b), h).astype(_BF)
                pltpu.make_async_copy(o_v.at[a:b, oq], o_hbm.at[a:b, oq], sem.at[0]).start()
        cols = []
        for b, nn in enumerate(_N2):
            for c in range(0, F, 128):
                slot, cc = (0, c) if c < H else (1 + (c - H) // lf, (c - H) % lf)
                cols.append((wt_v.at[slot], b * H + cc, b * F + c, (0, 16) if c < nn * 128 else (16,)))
        tail_chain(xb, gn, cols, t_out, None, _TREE)
        return jnp.minimum(gn + 2, 2 * (nm - 1))

    lax.fori_loop(0, nm, mloop, jnp.int32(2))
    keep = pltpu.make_async_copy(tall.at[1, 16:24, 0:128], keep_hbm, sem.at[1])
    keep.start()
    pltpu.make_async_copy(o_v, o_hbm, sem.at[0]).wait()
    keep.wait()


@jax.jit
def pallas_standalone__geglu_ffn__prompt_kernel(x, w_gate, w_up, w_down):
    B, S, D = x.shape
    F = w_gate.shape[1]
    M = B * S
    H = sum(_HEAD)
    lf = (F - H) // _NL
    ng = (M - _T0) // 128
    assert D == _KM + _KT and lf <= H
    assert (F - H) % (128 * _NL) == 0 and H % (128 * _NL) == 0
    assert (M - _T0) % _TS == 0 and (M - _T0) % (128 * _NL) == 0
    xT = x.reshape(M, D).T
    wdT = w_down.T
    outT, _ = pl.pallas_call(
        _kernel,
        in_specs=[pl.BlockSpec(memory_space=pl.ANY)] * 4,
        out_specs=[pl.BlockSpec(memory_space=pl.ANY)] * 2,
        out_shape=[jax.ShapeDtypeStruct((D, M), x.dtype), jax.ShapeDtypeStruct((8, 128), _F32)],
        scratch_shapes=[
            pltpu.VMEM((_NL + 1, D, _SLOTW), _BF),
            pltpu.VMEM((_NL + 1, D // 2, H), _U32),
            pltpu.VMEM((_NL + 1, D // 2, H), _U32),
            pltpu.VMEM((_NL, D // 2, H), _U32),
            pltpu.VMEM((_NL, D // 2, H // _NL), _U32),
            pltpu.VMEM((_T0, D), _BF), pltpu.VMEM((_T0, D), _BF),
            pltpu.VMEM((ng, 64, D), _U32), pltpu.VMEM((ng, 64, D), _U32),
            pltpu.VMEM((_NL, _T0, H // _NL), _BF),
            pltpu.VMEM((D, _T0), _F32),
            pltpu.VMEM((D, M), _BF),
            pltpu.VMEM((_NL + 1, _KT, 2 * H), _F32),
            pltpu.VMEM((_KT, 2 * lf), _F32),
            pltpu.VMEM((ng, _KT, 32, 128), _F32),
            pltpu.VMEM((2, _KT, 32, 128), _F32),
            pltpu.VMEM(((M - _T0) // _TS + 1, 64, 2 * F), _F32),
            pltpu.VMEM((16, 128), _F32),
            pltpu.SMEM((_NL,), jnp.int32),
            pltpu.SemaphoreType.DMA((1 + _XSPLIT + len(_HEAD) + _NL,)),
        ],
        compiler_params=pltpu.CompilerParams(
            vmem_limit_bytes=110 * 1024 * 1024,
            disable_bounds_checks=True,
            disable_semaphore_checks=True,
        ),
    )(xT, w_gate, w_up, wdT)
    return outT.T.reshape(B, S, D)
```

```python
import jax
import jax.numpy as jnp
from jax import lax
import jax.experimental.pallas as pl
import jax.experimental.pallas.tpu as pltpu

_NT = (((1,), (1,)), ((), ()))
_F32 = jnp.float32
_BF = jnp.bfloat16
_U32 = jnp.uint32
_C0 = 0.7978845608028654
_C1 = _C0 * 0.044715

_KM = 512
_KT = 64
_T0 = 512
_TS = 256
_HEAD = (128, 256, 640)
_NL = 4
_XSPLIT = 2
_SLOTW = 4096
_N2 = (32, 32)
_GC = 4
_TREE = (2, 8, 90)
_DSPLIT = (0, 448, 576)


def _act(g, uh):
    t = jnp.tanh(g * (_C0 + _C1 * (g * g)))
    return ((g * (1.0 + t)) * uh).astype(_BF)


def _half(x):
    return (x.astype(_F32) * 0.5).astype(_BF)


def _mo(v):
    return v if isinstance(v, int) else pl.multiple_of(v, 128)


def _dot(a, b):
    return jnp.dot(a, b, preferred_element_type=_F32)


def _dot_nt(a, b):
    return lax.dot_general(a, b, _NT, preferred_element_type=_F32)


def _cat(parts, axis):
    return parts[0] if len(parts) == 1 else jnp.concatenate(parts, axis=axis)


def _kernel(xT_hbm, wg_hbm, wu_hbm, wd_hbm, o_hbm, keep_hbm,
            buf, pg, pu, pd, pd0, x0_v, xu0_v, x_v, xu_v, h0_v, acc_v, o_v,
            wt_v, wts, xb, xb0, tall, m_v, z_s, sem):
    D, M = o_v.shape
    F = wg_hbm.shape[1]
    t0, ts, head, nl = _T0, _TS, _HEAD, _NL
    nh = len(head)
    hoff = [sum(head[:j]) for j in range(nh + 1)]
    H = hoff[-1]
    lf = (F - H) // nl
    hc = H // nl
    nm = (M - t0) // ts
    xp = t0 // _XSPLIT
    xr = (M - t0) // nl
    gpi = xr // 128
    hbm = dict(x=xT_hbm, g=wg_hbm, u=wu_hbm, d=wd_hbm)
    pos0 = dict(x=0, g=t0, u=t0 + H, xs=t0 + 2 * H)
    posl = dict(g=0, u=lf, d=2 * lf, d0=3 * lf, x=3 * lf + hc)

    def cp(k, off, size, slot, pos, s):
        return pltpu.make_async_copy(hbm[k].at[:, pl.ds(_mo(off), size)],
                                     buf.at[slot, :, pos:pos + size], sem.at[s])

    def x_cps(p):
        return [cp('x', p * xp, xp, 0, p * xp, 1 + p)]

    def head_cps(j):
        s = 1 + _XSPLIT + j
        cps = [cp(k, hoff[j], head[j], 0, pos0[k] + hoff[j], s) for k in 'gu']
        if j == nh - 1:
            cps.append(pltpu.make_async_copy(xT_hbm.at[_KM:D, t0:t0 + ts],
                                             buf.at[0, 0:_KT, pos0['xs']:pos0['xs'] + ts], sem.at[s]))
        return cps

    def loop_cps(j):
        s = 1 + _XSPLIT + nh + j
        return ([cp(k, H + j * lf, lf, 1 + j, posl[k], s) for k in 'gud']
                + [cp('d', j * hc, hc, 1 + j, posl['d0'], s),
                   cp('x', t0 + j * xr, xr, 1 + j, posl['x'], s)])

    def rd0(k, off, size, r0=0, r1=D):
        return buf[0, r0:r1, pos0[k] + off:pos0[k] + off + size]

    def rdl(k, j, size, r0=0, r1=D):
        return buf[1 + j, r0:r1, posl[k]:posl[k] + size]

    def keep_packed(ref, slot, off, w):
        ref[slot, :, off:off + w.shape[1]] = pltpu.bitcast(w, _U32)
        return w

    def rdm(k, c0, c1, r0=0, r1=D):
        if k == 'd':
            segs = [(pd0, s, s * hc, hc) for s in range(nl)] + [(pd, s, H + s * lf, lf) for s in range(nl)]
        else:
            ref = pg if k == 'g' else pu
            segs = [(ref, 0, 0, H)] + [(ref, 1 + s, H + s * lf, lf) for s in range(nl)]
        parts = []
        for ref, slot, st, n in segs:
            a, b = max(c0, st), min(c1, st + n)
            if a < b:
                parts.append(ref[slot, r0 // 2:r1 // 2, a - st:b - st])
        return pltpu.bitcast(_cat(parts, 1), _BF)

    for p in range(_XSPLIT):
        for c in x_cps(p):
            c.start()
    for j in range(nh):
        for c in head_cps(j):
            c.start()
    for j in range(nl):
        for c in loop_cps(j):
            c.start()

    acc_v[...] = jnp.zeros_like(acc_v)
    m_v[...] = jnp.zeros_like(m_v)
    for j in range(nl):
        z_s[j] = 0

    def build_xb(xtl, ngrp, dst, g0):
        never = m_v[0:8, :] > 0
        zero = jnp.zeros((8, 128), _F32)
        prev = None
        for k in range(_KT):
            col = jnp.broadcast_to(xtl[:, k:k + 1], (32 * ngrp, 128))
            for q in range(ngrp):
                for r in range(0, 32, 8):
                    v = col[32 * q + r:32 * q + r + 8]
                    prev = v if prev is None else v + jnp.where(never, prev, zero)
                    dst[g0 + q, k, r:r + 8, :] = prev

    def tail_chain(xsrc, g0, cols, dst, prev=None, tsch=(0, 0, 0)):
        never = m_v[...] > 0
        left = sum(2 * len(c[3]) for c in cols)
        xq = [xsrc.at[g0 + q] for q in range(2)]
        for wref, wc, col, units in cols:
            cs = pl.ds(_mo(col), 128)
            for q in range(2):
                for rr in units:
                    tree = tsch[1] if left <= tsch[2] else tsch[0]
                    left -= 1

                    def prod(k):
                        return xq[q][k, rr:rr + 16, :] * wref[pl.ds(k, 1), wc:wc + 128]

                    def singles(lo, hi, a):
                        return lax.fori_loop(lo, hi, lambda k, b: b + prod(k), a, unroll=True)

                    acc = prod(0) if prev is None else jnp.where(never, prev, prod(0))
                    if tree == 0:
                        acc = singles(1, _KT, acc)
                    for t in range(tree):
                        k0, gs = t * (_KT // tree), _KT // tree
                        pa = prod(k0 + 1)
                        acc = acc + (pa + prod(k0 + 2))
                        acc = singles(k0 + 3, min(k0 + gs + 1, _KT), acc)
                    dst[32 * q + rr:32 * q + rr + 16, cs] = acc
                    prev = acc
        return prev

    for p in range(_XSPLIT):
        for c in x_cps(p):
            c.wait()
        xt = rd0('x', p * xp, xp).T
        x0_v[p * xp:(p + 1) * xp, :] = xt
        xu0_v[p * xp:(p + 1) * xp, :] = _half(xt)

    for j in range(nh):
        for c in head_cps(j):
            c.wait()
        nsp = 2 if (head[j] // 128) % 2 == 1 else 1
        rp = t0 // nsp
        wg_c = keep_packed(pg, 0, hoff[j], rd0('g', hoff[j], head[j]))
        wu_c = keep_packed(pu, 0, hoff[j], rd0('u', hoff[j], head[j]))
        for p in range(nsp):
            rows = slice(p * rp, (p + 1) * rp)
            g = _dot(x0_v[rows, :], wg_c)
            u = _dot(xu0_v[rows, :], wu_c)
            for c in range(hoff[j], hoff[j + 1], 128):
                cl = c - hoff[j]
                h0_v[c // hc, rows, c % hc:c % hc + 128] = _act(g[:, cl:cl + 128], u[:, cl:cl + 128])
        wt_v[0, :, hoff[j]:hoff[j + 1]] = rd0('g', hoff[j], head[j], _KM, D).astype(_F32)
        wt_v[0, :, H + hoff[j]:H + hoff[j + 1]] = rd0('u', hoff[j], head[j], _KM, D).astype(_F32) * 0.5
        if j == nh - 1:
            xs = rd0('xs', 0, ts, 0, _KT).astype(_F32).T
            xs = jnp.concatenate([xs[96:128], xs[224:256]], axis=0)
            tall[0, :, 0:H] = _dot(xs.astype(_BF), rd0('g', 0, H, _KM, D))
            tall[0, :, F:F + H] = _dot((xs * 0.5).astype(_BF), rd0('u', 0, H, _KM, D))
            build_xb(xs, 2, xb0, 0)

    def ploop(j, jc):
        g = _dot(x0_v[...], keep_packed(pg, 1 + j, 0, rdl('g', j, lf)))
        u = _dot(xu0_v[...], keep_packed(pu, 1 + j, 0, rdl('u', j, lf)))
        h = _act(g, u)
        y = _dot_nt(keep_packed(pd0, j, 0, rdl('d0', j, hc)), h0_v[j])
        y = y + _dot_nt(keep_packed(pd, j, 0, rdl('d', j, lf)), h)
        a = acc_v[...] + y
        acc_v[...] = a
        o_v[:, 0:t0] = a.astype(_BF)
        tg = rdl('g', jc, lf, _KM, D).astype(_F32)
        tu = rdl('u', jc, lf, _KM, D).astype(_F32) * 0.5
        wt_v[1 + jc, :, 0:lf] = tg
        wt_v[1 + jc, :, H:H + lf] = tu
        xin = rdl('x', jc, xr)
        wts[:, 0:lf] = tg
        wts[:, lf:2 * lf] = tu
        cols = [(wts, b * lf + c, b * F + H + jc * lf + c, (0, 16)) for b in range(2) for c in range(0, lf, 128)]
        gate = wts[pl.ds(pl.multiple_of(z_s[jc], 8), 16), 0:128]
        last = tail_chain(xb0, 0, cols, tall.at[0], gate)
        mk = jnp.concatenate([m_v[...] > 0] * gpi, axis=1)
        lb = jnp.concatenate([last.astype(_BF)] * gpi, axis=1)
        parts = []
        for r in range(0, D, 128):
            parts.append(jnp.where(mk, lb, xin[r:r + 16]))
            parts.append(xin[r + 16:min(r + 128, D)])
        xt = jnp.concatenate(parts, axis=0).T
        for q in range(gpi):
            x_v[jc * gpi + q] = pltpu.bitcast(xt[128 * q:128 * q + 128], _U32)
            xu_v[jc * gpi + q] = pltpu.bitcast(_half(xt[128 * q:128 * q + 128]), _U32)
        xtl = jnp.concatenate([x_v[jc * gpi + q, 48:64, _KM:] for q in range(gpi)], axis=0)
        build_xb(pltpu.bitcast(xtl, _BF).astype(_F32), gpi, xb, jc * gpi)

        @pl.when(j + 1 < nl)
        def _():
            for c in loop_cps(j + 1):
                c.wait()

        return jnp.minimum(jc + 1, nl - 1)

    for c in loop_cps(0):
        c.wait()
    lax.fori_loop(0, nl, ploop, jnp.int32(0))
    pltpu.make_async_copy(o_v.at[:, 0:t0], o_hbm.at[:, 0:t0], sem.at[0]).start()

    def mloop(i, gn):
        r0 = pl.multiple_of(i * ts, 128)
        t_in, t_out = tall.at[i], tall.at[i + 1]

        def proj(ref, k, base, nn, ca, cb):
            xa, xc = ref[2 * i], ref[2 * i + 1]

            def rows(n, c0, c1):
                return pltpu.bitcast(jnp.concatenate([xa[0:n // 2, c0:c1], xc[0:n // 2, c0:c1]], axis=0), _BF)

            c2 = min(max(nn * 128, ca), cb)
            inits = []
            if c2 > ca:
                ta = _dot(rows(96, _KM, D), rdm(k, ca, c2, _KM, D))
                inits.append(jnp.concatenate([ta[0:96], t_in[0:32, base + ca:base + c2],
                                              ta[96:192], t_in[32:64, base + ca:base + c2]], axis=0))
            if c2 < cb:
                ta = _dot(rows(112, _KM, D), rdm(k, c2, cb, _KM, D))
                inits.append(jnp.concatenate([ta[0:112], t_in[16:32, base + c2:base + cb],
                                              ta[112:224], t_in[48:64, base + c2:base + cb]], axis=0))
            return _dot(rows(128, 0, _KM), rdm(k, ca, cb, 0, _KM)) + _cat(inits, 1)

        hs = [[], []]
        for ca in range(0, F, _GC * 128):
            cb = min(ca + _GC * 128, F)
            g = proj(x_v, 'g', 0, _N2[0], ca, cb)
            u = proj(xu_v, 'u', F, _N2[1], ca, cb)
            for q in range(2):
                hs[q].append(_act(g[q * 128:(q + 1) * 128], u[q * 128:(q + 1) * 128]))
        for q in range(2):
            h = _cat(hs[q], 1)
            oq = pl.ds(pl.multiple_of(t0 + r0 + q * 128, 128), 128)
            cuts = _DSPLIT if q == 1 else (0, D)
            for a, b in zip(cuts[:-1], cuts[1:]):
                o_v[a:b, oq] = _dot_nt(rdm('d', 0, F, a, b), h).astype(_BF)
                pltpu.make_async_copy(o_v.at[a:b, oq], o_hbm.at[a:b, oq], sem.at[0]).start()
        cols = []
        for b, nn in enumerate(_N2):
            for c in range(0, F, 128):
                slot, cc = (0, c) if c < H else (1 + (c - H) // lf, (c - H) % lf)
                cols.append((wt_v.at[slot], b * H + cc, b * F + c, (0, 16) if c < nn * 128 else (16,)))
        tail_chain(xb, gn, cols, t_out, None, _TREE)
        return jnp.minimum(gn + 2, 2 * (nm - 1))

    lax.fori_loop(0, nm, mloop, jnp.int32(2))
    keep = pltpu.make_async_copy(tall.at[1, 16:24, 0:128], keep_hbm, sem.at[1])
    keep.start()
    pltpu.make_async_copy(o_v, o_hbm, sem.at[0]).wait()
    keep.wait()


@jax.jit
def pallas_standalone__geglu_ffn__prompt_kernel(x, w_gate, w_up, w_down):
    B, S, D = x.shape
    F = w_gate.shape[1]
    M = B * S
    H = sum(_HEAD)
    lf = (F - H) // _NL
    ng = (M - _T0) // 128
    assert D == _KM + _KT and lf <= H
    assert (F - H) % (128 * _NL) == 0 and H % (128 * _NL) == 0
    assert (M - _T0) % _TS == 0 and (M - _T0) % (128 * _NL) == 0
    xT = x.reshape(M, D).T
    wdT = w_down.T
    outT, _ = pl.pallas_call(
        _kernel,
        in_specs=[pl.BlockSpec(memory_space=pl.ANY)] * 4,
        out_specs=[pl.BlockSpec(memory_space=pl.ANY)] * 2,
        out_shape=[jax.ShapeDtypeStruct((D, M), x.dtype), jax.ShapeDtypeStruct((8, 128), _F32)],
        scratch_shapes=[
            pltpu.VMEM((_NL + 1, D, _SLOTW), _BF),
            pltpu.VMEM((_NL + 1, D // 2, H), _U32),
            pltpu.VMEM((_NL + 1, D // 2, H), _U32),
            pltpu.VMEM((_NL, D // 2, H), _U32),
            pltpu.VMEM((_NL, D // 2, H // _NL), _U32),
            pltpu.VMEM((_T0, D), _BF), pltpu.VMEM((_T0, D), _BF),
            pltpu.VMEM((ng, 64, D), _U32), pltpu.VMEM((ng, 64, D), _U32),
            pltpu.VMEM((_NL, _T0, H // _NL), _BF),
            pltpu.VMEM((D, _T0), _F32),
            pltpu.VMEM((D, M), _BF),
            pltpu.VMEM((_NL + 1, _KT, 2 * H), _F32),
            pltpu.VMEM((_KT, 2 * lf), _F32),
            pltpu.VMEM((ng, _KT, 32, 128), _F32),
            pltpu.VMEM((2, _KT, 32, 128), _F32),
            pltpu.VMEM(((M - _T0) // _TS + 1, 64, 2 * F), _F32),
            pltpu.VMEM((16, 128), _F32),
            pltpu.SMEM((_NL,), jnp.int32),
            pltpu.SemaphoreType.DMA((1 + _XSPLIT + len(_HEAD) + _NL,)),
        ],
        compiler_params=pltpu.CompilerParams(
            vmem_limit_bytes=110 * 1024 * 1024,
            disable_bounds_checks=True,
            disable_semaphore_checks=True,
        ),
    )(xT, w_gate, w_up, wdT)
    return outT.T.reshape(B, S, D)
```

```python
import jax
import jax.numpy as jnp
from jax import lax
import jax.experimental.pallas as pl
import jax.experimental.pallas.tpu as pltpu

_NT = (((1,), (1,)), ((), ()))
_F32 = jnp.float32
_BF = jnp.bfloat16
_U32 = jnp.uint32
_C0 = 0.7978845608028654
_C1 = _C0 * 0.044715

_KM = 512
_KT = 64
_KG = 8
_T0 = 512
_TS = 256
_NL = 4
_SLOTW = 4096
_EA = 48
_NF1 = 10
_N2 = (32, 24)
_GC = 4
_PW = 1152
_TREE = (2, 8, 90)
_DSPLIT = (0, 448, 576)


def _act(g, uh):
    t = jnp.tanh(g * (_C0 + _C1 * (g * g)))
    return ((g * (1.0 + t)) * uh).astype(_BF)


def _half(x):
    return (x.astype(_F32) * 0.5).astype(_BF)


def _mo(v):
    return v if isinstance(v, int) else pl.multiple_of(v, 128)


def _dot(a, b):
    return jnp.dot(a, b, preferred_element_type=_F32)


def _dot_nt(a, b):
    return lax.dot_general(a, b, _NT, preferred_element_type=_F32)


def _cat(parts, axis):
    return parts[0] if len(parts) == 1 else jnp.concatenate(parts, axis=axis)


def _bf(x):
    return pltpu.bitcast(x, _BF)


def _u32(x):
    return pltpu.bitcast(x, _U32)


def _kernel(xT_hbm, wg_hbm, wu_hbm, wd_hbm, o_hbm, keep_hbm,
            buf, pg, pu, pd, x0_v, xu0_v, x_v, xu_v, xe_v, acc_v, o_v, wt_v, xb, xb0, tall, te_v, m_v, sem):
    D, M = o_v.shape
    F = wg_hbm.shape[1]
    t0, ts, nl = _T0, _TS, _NL
    lf = F // nl
    nm = (M - t0) // ts
    xr = (M - t0) // nl
    gpi = xr // 128
    ng = (M - t0) // 128
    ne = 96 - _EA
    f1 = _NF1 * 128
    hbm = dict(x=xT_hbm, g=wg_hbm, u=wu_hbm, d=wd_hbm)
    posl = dict(g=0, u=lf, d=2 * lf, x=3 * lf)
    XT = t0
    packed = dict(g=pg, u=pu, d=pd)

    def cp(k, r0, r1, off, size, slot, dr0, pos, s):
        return pltpu.make_async_copy(hbm[k].at[r0:r1, pl.ds(_mo(off), size)],
                                     buf.at[slot, dr0:dr0 + r1 - r0, pos:pos + size], sem.at[s])

    def band(k, j):
        return _KT * (1 + 2 * j + (k == 'u'))

    def tail_cps(c0, c1, s):
        cps = []
        for j in range(nl):
            a, b = max(c0, j * lf), min(c1, (j + 1) * lf)
            if a < b:
                cps += [cp(k, _KM, D, a, b - a, 0, band(k, j), XT + a - j * lf, s) for k in 'gu']
        return cps

    f1_cps = [cp('x', _KM, D, t0, M - t0, 0, 0, XT, 1)] + tail_cps(0, f1, 1)
    f2_cps = [cp('x', 0, D, 0, t0, 0, 0, 0, 2)] + tail_cps(f1, F, 2)

    def loop_cps(j):
        s, slot = 3 + j % 2, 1 + j % 2
        return ([cp(k, 0, _KM, j * lf, lf, slot, 0, posl[k], s) for k in 'gu']
                + [cp('d', 0, D, j * lf, lf, slot, 0, posl['d'], s),
                   cp('x', 0, D, t0 + j * xr, xr, slot, 0, posl['x'], s)])

    def fresh(k, j, rows):
        w = buf[1 + j % 2, 0:rows, posl[k]:posl[k] + lf]
        packed[k][j, 0:rows // 2, 0:lf] = _u32(w)
        return w

    def rdm(k, c0, c1, r0=0, r1=D):
        parts = []
        for s in range(nl):
            a, b = max(c0, s * lf), min(c1, (s + 1) * lf)
            if a < b:
                parts.append(packed[k][s, r0 // 2:r1 // 2, a - s * lf:b - s * lf])
        return _bf(_cat(parts, 1))

    for c in f1_cps + f2_cps + loop_cps(0) + loop_cps(1):
        c.start()

    acc_v[...] = jnp.zeros_like(acc_v)
    m_v[...] = jnp.zeros_like(m_v)

    def build_xb(xtl, ngrp, dst, g0):
        never = m_v[0:8, :] > 0
        zero = jnp.zeros((8, 128), _F32)
        prev = None
        for k in range(_KT):
            col = jnp.broadcast_to(xtl[:, k:k + 1], (32 * ngrp, 128))
            for q in range(ngrp):
                for r in range(0, 32, 8):
                    v = col[32 * q + r:32 * q + r + 8]
                    prev = v if prev is None else v + jnp.where(never, prev, zero)
                    dst[g0 + q, k, r:r + 8, :] = prev

    def tail_chain(xsrc, g0, cols, dst, prev=None, tsch=(0, 0, 0)):
        never = m_v[...] > 0
        left = sum(2 * len(c[3]) for c in cols)
        xq = [xsrc.at[g0 + q] for q in range(2)]
        for wref, wc, col, units in cols:
            cs = pl.ds(_mo(col), 128)
            wk = {}
            for q in range(2):
                for rr in units:
                    tree = tsch[1] if left <= tsch[2] else tsch[0]
                    left -= 1
                    pairs = {t * (_KT // tree) for t in range(tree)}
                    acc = None
                    for k0 in range(0, _KT, _KG):
                        x8 = xq[q][k0:k0 + _KG, rr:rr + 16, :]
                        if k0 not in wk:
                            wk[k0] = jnp.concatenate(
                                [lax.broadcast_in_dim(wref[k:k + 1, wc:wc + 128], (1, 16, 128), (1, 2))
                                 for k in range(k0, k0 + _KG)], axis=0)
                        p = x8 * wk[k0]
                        terms, lo = [], 0
                        if acc is not None:
                            terms.append(acc[None])
                        elif prev is not None:
                            terms.append(jnp.where(never, prev, p[0])[None])
                            lo = 1
                        if k0 in pairs:
                            if lo < 1:
                                terms.append(p[0:1])
                            terms.append(p[1:2] + p[2:3])
                            lo = 3
                        terms.append(p[lo:] if lo else p)
                        acc = jnp.sum(_cat(terms, 0), axis=0)
                    dst[32 * q + rr:32 * q + rr + 16, cs] = acc
                    prev = acc
        return prev

    def filler(lhs, c0, c1):
        for j in range(nl):
            ca, cb = max(c0, j * lf) - j * lf, min(c1, (j + 1) * lf) - j * lf
            if ca >= cb:
                continue
            for b, k in enumerate('gu'):
                wp = _u32(buf[0, band(k, j):band(k, j) + _KT, XT + ca:XT + cb])
                packed[k][j, _KM // 2:D // 2, ca:cb] = wp
                w = _bf(wp)
                te = _dot(lhs[b], w)
                gc0 = b * F + j * lf
                for t in range(nm):
                    te_v[t, :, gc0 + ca:gc0 + cb] = te[2 * ne * t:2 * ne * (t + 1)]
                wt_v[j, :, b * lf + ca:b * lf + cb] = w.astype(_F32) * 0.5 if b else w.astype(_F32)

    for c in f1_cps:
        c.wait()
    xt = buf[0, 0:_KT, XT:XT + M - t0].T
    xe = jnp.concatenate([xt[128 * q + _EA:128 * q + 96] for q in range(ng)], axis=0)
    lhs = (xe, _half(xe))
    xe_v[0] = lhs[0]
    xe_v[1] = lhs[1]
    xe_v[2, 0:64, :] = jnp.concatenate([xt[96:128], xt[224:256]], axis=0)
    filler(lhs, 0, f1)

    for c in f2_cps:
        c.wait()
    filler((xe_v[0], xe_v[1]), f1, F)
    x0t = buf[0, :, 0:t0].T
    x0_v[...] = _u32(x0t)
    xu0_v[...] = _u32(_half(x0t))
    build_xb(xe_v[2, 0:64, :].astype(_F32), 2, xb0, 0)

    def ploop(j, jc):
        def wfull(k):
            return jnp.concatenate([fresh(k, j, _KM), _bf(packed[k][j, _KM // 2:D // 2, 0:lf])], axis=0)

        g = _dot(_bf(x0_v[...]), wfull('g'))
        u = _dot(_bf(xu0_v[...]), wfull('u'))
        a = acc_v[...] + _dot_nt(fresh('d', j, D), _act(g, u))
        acc_v[...] = a
        o_v[:, 0:t0] = a.astype(_BF)
        xin = buf[1 + jc % 2, :, posl['x']:posl['x'] + xr]
        wq = wt_v.at[jc]
        cols = [(wq, b * lf + c, b * F + jc * lf + c, (0, 16)) for b in range(2) for c in range(0, lf, 128)]
        last = tail_chain(xb0, 0, cols, tall.at[0])
        mk = jnp.concatenate([m_v[...] > 0] * gpi, axis=1)
        lb = jnp.concatenate([last.astype(_BF)] * gpi, axis=1)
        parts = []
        for r in range(0, D, 128):
            parts.append(jnp.where(mk, lb, xin[r:r + 16]))
            parts.append(xin[r + 16:min(r + 128, D)])
        xt = jnp.concatenate(parts, axis=0).T
        for q in range(gpi):
            x_v[jc * gpi + q] = _u32(xt[128 * q:128 * q + 128])
            xu_v[jc * gpi + q] = _u32(_half(xt[128 * q:128 * q + 128]))
        xtl = jnp.concatenate([x_v[jc * gpi + q, 48:64, _KM:] for q in range(gpi)], axis=0)
        build_xb(_bf(xtl).astype(_F32), gpi, xb, jc * gpi)

        @pl.when(j + 1 < nl)
        def _():
            for c in loop_cps(j + 1):
                c.wait()

        @pl.when(j + 2 < nl)
        def _():
            for c in loop_cps(j + 2):
                c.start()

        return jnp.minimum(jc + 1, nl - 1)

    for c in loop_cps(0):
        c.wait()
    lax.fori_loop(0, nl, ploop, jnp.int32(0))
    pltpu.make_async_copy(o_v.at[:, 0:t0], o_hbm.at[:, 0:t0], sem.at[0]).start()

    def mloop(i, gn):
        r0 = pl.multiple_of(i * ts, 128)
        t_in, t_out, t_e = tall.at[i], tall.at[i + 1], te_v.at[i]

        def proj(ref, k, base, nn, ca, cb):
            xs = (ref[2 * i], ref[2 * i + 1])
            c2 = min(max(nn * 128, ca), cb)
            inits = []
            for lo, hi, two in ((ca, c2, True), (c2, cb, False)):
                if lo >= hi:
                    continue
                segs = [(0, _EA)] + ([] if two else [(96, 112)])
                na = sum(b - a for a, b in segs)
                ta = _dot(_bf(_cat([x[a // 2:b // 2, _KM:] for x in xs for a, b in segs], 0)), rdm(k, lo, hi, _KM, D))
                cs = slice(base + lo, base + hi)
                parts = []
                for q in range(2):
                    parts.append(ta[q * na:q * na + _EA])
                    parts.append(t_e[q * ne:(q + 1) * ne, cs])
                    if two:
                        parts.append(t_in[32 * q:32 * q + 32, cs])
                    else:
                        parts.append(ta[q * na + _EA:(q + 1) * na])
                        parts.append(t_in[32 * q + 16:32 * q + 32, cs])
                inits.append(jnp.concatenate(parts, axis=0))
            xm = _bf(jnp.concatenate([x[:, 0:_KM] for x in xs], axis=0))
            return _dot(xm, rdm(k, ca, cb, 0, _KM)) + _cat(inits, 1)

        hs = [[], []]
        for ca in range(0, F, _GC * 128):
            cb = min(ca + _GC * 128, F)
            g = proj(x_v, 'g', 0, _N2[0], ca, cb)
            u = proj(xu_v, 'u', F, _N2[1], ca, cb)
            for q in range(2):
                hs[q].append(_act(g[q * 128:(q + 1) * 128], u[q * 128:(q + 1) * 128]))
        for q in range(2):
            h = _cat(hs[q], 1)
            oq = pl.ds(pl.multiple_of(t0 + r0 + q * 128, 128), 128)
            cuts = _DSPLIT if q == 1 else (0, D)
            for a, b in zip(cuts[:-1], cuts[1:]):
                o_v[a:b, oq] = _dot_nt(rdm('d', 0, F, a, b), h).astype(_BF)
                pltpu.make_async_copy(o_v.at[a:b, oq], o_hbm.at[a:b, oq], sem.at[0]).start()
        cols = [(wt_v.at[c // lf], b * lf + c % lf, b * F + c, (0, 16) if c < nn * 128 else (16,))
                for b, nn in enumerate(_N2) for c in range(0, F, 128)]
        tail_chain(xb, gn, cols, t_out, None, _TREE)
        return jnp.minimum(gn + 2, 2 * (nm - 1))

    lax.fori_loop(0, nm, mloop, jnp.int32(2))
    keep = pltpu.make_async_copy(tall.at[1, 16:24, 0:128], keep_hbm, sem.at[1])
    keep.start()
    pltpu.make_async_copy(o_v, o_hbm, sem.at[0]).wait()
    keep.wait()


@jax.jit
def pallas_standalone__geglu_ffn__prompt_kernel(x, w_gate, w_up, w_down):
    B, S, D = x.shape
    F = w_gate.shape[1]
    M = B * S
    lf = F // _NL
    ng = (M - _T0) // 128
    ne = 96 - _EA
    xT = x.reshape(M, D).T
    wdT = w_down.T
    outT, _ = pl.pallas_call(
        _kernel,
        in_specs=[pl.BlockSpec(memory_space=pl.ANY)] * 4,
        out_specs=[pl.BlockSpec(memory_space=pl.ANY)] * 2,
        out_shape=[jax.ShapeDtypeStruct((D, M), x.dtype), jax.ShapeDtypeStruct((8, 128), _F32)],
        scratch_shapes=[
            pltpu.VMEM((3, D, _SLOTW), _BF),
            pltpu.VMEM((_NL, D // 2, _PW), _U32), pltpu.VMEM((_NL, D // 2, _PW), _U32), pltpu.VMEM((_NL, D // 2, _PW), _U32),
            pltpu.VMEM((_T0 // 2, D), _U32), pltpu.VMEM((_T0 // 2, D), _U32),
            pltpu.VMEM((ng, 64, D), _U32), pltpu.VMEM((ng, 64, D), _U32),
            pltpu.VMEM((3, ng * ne, _KT), _BF),
            pltpu.VMEM((D, _T0), _F32),
            pltpu.VMEM((D, M), _BF),
            pltpu.VMEM((_NL, _KT, 4096), _F32),
            pltpu.VMEM((ng, _KT, 32, 128), _F32),
            pltpu.VMEM((2, _KT, 32, 128), _F32),
            pltpu.VMEM(((M - _T0) // _TS + 1, 64, 2 * F), _F32),
            pltpu.VMEM(((M - _T0) // _TS, 2 * ne, 2 * F), _F32),
            pltpu.VMEM((16, 128), _F32),
            pltpu.SemaphoreType.DMA((5,)),
        ],
        compiler_params=pltpu.CompilerParams(
            vmem_limit_bytes=116 * 1024 * 1024,
            disable_bounds_checks=True,
            disable_semaphore_checks=True,
        ),
    )(xT, w_gate, w_up, wdT)
    return outT.T.reshape(B, S, D)
```

```python
import jax
import jax.numpy as jnp
from jax import lax
import jax.experimental.pallas as pl
import jax.experimental.pallas.tpu as pltpu

_NT = (((1,), (1,)), ((), ()))
_F32 = jnp.float32
_BF = jnp.bfloat16
_U32 = jnp.uint32
_C0 = 0.7978845608028654
_C1 = _C0 * 0.044715

_KM = 512
_KT = 64
_KG = 8
_T0 = 512
_TS = 256
_NL = 4
_SLOTW = 3840
_EA = 48
_NF1 = 10
_N2 = (33, 24)
_GC = 4
_TREE = (2, 8, 90)
_DSPLIT = (0, 448, 576)


def _act(g, uh):
    t = jnp.tanh(g * (_C0 + _C1 * (g * g)))
    return ((g * (1.0 + t)) * uh).astype(_BF)


def _half(x):
    return (x.astype(_F32) * 0.5).astype(_BF)


def _mo(v):
    return v if isinstance(v, int) else pl.multiple_of(v, 128)


def _dot(a, b):
    return jnp.dot(a, b, preferred_element_type=_F32)


def _dot_nt(a, b):
    return lax.dot_general(a, b, _NT, preferred_element_type=_F32)


def _cat(parts, axis):
    return parts[0] if len(parts) == 1 else jnp.concatenate(parts, axis=axis)


def _bf(x):
    return pltpu.bitcast(x, _BF)


def _u32(x):
    return pltpu.bitcast(x, _U32)


def _kernel(xT_hbm, wg_hbm, wu_hbm, wd_hbm, o_hbm, keep_hbm,
            buf, pg, pu, pd, x0_v, xu0_v, x_v, xu_v, xe_v, acc_v, o_v, wt_v, xb, xb0, tall, te_v, m_v, sem):
    D, M = o_v.shape
    F = wg_hbm.shape[1]
    t0, ts, nl = _T0, _TS, _NL
    lf = F // nl
    nm = (M - t0) // ts
    xr = (M - t0) // nl
    gpi = xr // 128
    ng = (M - t0) // 128
    ne = 96 - _EA
    f1 = _NF1 * 128
    hbm = dict(x=xT_hbm, g=wg_hbm, u=wu_hbm, d=wd_hbm)
    posl = dict(g=0, u=lf, d=2 * lf, x=3 * lf)
    XT = t0
    packed = dict(g=pg, u=pu, d=pd)

    def cp(k, r0, r1, off, size, slot, dr0, pos, s):
        return pltpu.make_async_copy(hbm[k].at[r0:r1, pl.ds(_mo(off), size)],
                                     buf.at[slot, dr0:dr0 + r1 - r0, pos:pos + size], sem.at[s])

    def band(k, j):
        return _KT * (1 + 2 * j + (k == 'u'))

    def tail_cps(c0, c1, s):
        cps = []
        for j in range(nl):
            a, b = max(c0, j * lf), min(c1, (j + 1) * lf)
            if a < b:
                cps += [cp(k, _KM, D, a, b - a, 0, band(k, j), XT + a - j * lf, s) for k in 'gu']
        return cps

    f1_cps = [cp('x', _KM, D, t0, M - t0, 0, 0, XT, 1)] + tail_cps(0, f1, 1)
    f2_cps = [cp('x', 0, D, 0, t0, 0, 0, 0, 2)] + tail_cps(f1, F, 2)

    def loop_cps(j):
        s, slot = 3 + j, 1 + j
        return ([cp(k, 0, _KM, j * lf, lf, slot, 0, posl[k], s) for k in 'gu']
                + [cp('d', 0, D, j * lf, lf, slot, 0, posl['d'], s),
                   cp('x', 0, D, t0 + j * xr, xr, slot, 0, posl['x'], s)])

    def fresh(k, j, rows):
        w = buf[1 + j, 0:rows, posl[k]:posl[k] + lf]
        packed[k][j, 0:rows // 2, 0:lf] = _u32(w)
        return w

    def rdm(k, c0, c1, r0=0, r1=D):
        parts = []
        for s in range(nl):
            a, b = max(c0, s * lf), min(c1, (s + 1) * lf)
            if a < b:
                parts.append(packed[k][s, r0 // 2:r1 // 2, a - s * lf:b - s * lf])
        return _bf(_cat(parts, 1))

    for c in f1_cps + f2_cps + [c_ for j in range(nl) for c_ in loop_cps(j)]:
        c.start()

    acc_v[...] = jnp.zeros_like(acc_v)
    m_v[...] = jnp.zeros_like(m_v)

    def build_xb(xtl, ngrp, dst, g0):
        never = m_v[0:8, :] > 0
        zero = jnp.zeros((8, 128), _F32)
        prev = None
        for k in range(_KT):
            col = jnp.broadcast_to(xtl[:, k:k + 1], (32 * ngrp, 128))
            for q in range(ngrp):
                for r in range(0, 32, 8):
                    v = col[32 * q + r:32 * q + r + 8]
                    prev = v if prev is None else v + jnp.where(never, prev, zero)
                    dst[g0 + q, k, r:r + 8, :] = prev

    def tail_chain(xsrc, g0, cols, dst, prev=None, tsch=(0, 0, 0)):
        never = m_v[...] > 0
        left = sum(2 * len(c[3]) for c in cols)
        xq = [xsrc.at[g0 + q] for q in range(2)]
        for wref, wc, col, units in cols:
            cs = pl.ds(_mo(col), 128)
            wk = {}
            for q in range(2):
                for rr in units:
                    tree = tsch[1] if left <= tsch[2] else tsch[0]
                    left -= 1
                    pairs = {t * (_KT // tree) for t in range(tree)}
                    acc = None
                    for k0 in range(0, _KT, _KG):
                        x8 = xq[q][k0:k0 + _KG, rr:rr + 16, :]
                        if k0 not in wk:
                            wk[k0] = jnp.concatenate(
                                [lax.broadcast_in_dim(wref[k:k + 1, wc:wc + 128], (1, 16, 128), (1, 2))
                                 for k in range(k0, k0 + _KG)], axis=0)
                        p = x8 * wk[k0]
                        terms, lo = [], 0
                        if acc is not None:
                            terms.append(acc[None])
                        elif prev is not None:
                            terms.append(jnp.where(never, prev, p[0])[None])
                            lo = 1
                        if k0 in pairs:
                            if lo < 1:
                                terms.append(p[0:1])
                            terms.append(p[1:2] + p[2:3])
                            lo = 3
                        terms.append(p[lo:] if lo else p)
                        acc = jnp.sum(_cat(terms, 0), axis=0)
                    dst[32 * q + rr:32 * q + rr + 16, cs] = acc
                    prev = acc
        return prev

    def filler(lhs, c0, c1):
        for j in range(nl):
            ca, cb = max(c0, j * lf) - j * lf, min(c1, (j + 1) * lf) - j * lf
            if ca >= cb:
                continue
            for b, k in enumerate('gu'):
                wp = _u32(buf[0, band(k, j):band(k, j) + _KT, XT + ca:XT + cb])
                packed[k][j, _KM // 2:D // 2, ca:cb] = wp
                w = _bf(wp)
                te = _dot(lhs[b], w)
                gc0 = b * F + j * lf
                for t in range(nm):
                    te_v[t, :, gc0 + ca:gc0 + cb] = te[2 * ne * t:2 * ne * (t + 1)]
                wt_v[j, :, b * lf + ca:b * lf + cb] = w.astype(_F32) * 0.5 if b else w.astype(_F32)

    for c in f1_cps:
        c.wait()
    xt = buf[0, 0:_KT, XT:XT + M - t0].T
    xe = jnp.concatenate([xt[128 * q + _EA:128 * q + 96] for q in range(ng)], axis=0)
    lhs = (xe, _half(xe))
    xe_v[0] = lhs[0]
    xe_v[1] = lhs[1]
    xe_v[2, 0:64, :] = jnp.concatenate([xt[96:128], xt[224:256]], axis=0)
    filler(lhs, 0, f1)

    for c in f2_cps:
        c.wait()
    filler((xe_v[0], xe_v[1]), f1, F)
    x0t = buf[0, :, 0:t0].T
    x0_v[...] = _u32(x0t)
    xu0_v[...] = _u32(_half(x0t))
    build_xb(xe_v[2, 0:64, :].astype(_F32), 2, xb0, 0)

    def ploop(j, jc):
        def wfull(k):
            return jnp.concatenate([fresh(k, j, _KM), _bf(packed[k][j, _KM // 2:D // 2, 0:lf])], axis=0)

        g = _dot(_bf(x0_v[...]), wfull('g'))
        u = _dot(_bf(xu0_v[...]), wfull('u'))
        a = acc_v[...] + _dot_nt(fresh('d', j, D), _act(g, u))
        acc_v[...] = a
        o_v[:, 0:t0] = a.astype(_BF)
        xin = buf[1 + jc, :, posl['x']:posl['x'] + xr]
        wq = wt_v.at[jc]
        cols = [(wq, b * lf + c, b * F + jc * lf + c, (0, 16)) for b in range(2) for c in range(0, lf, 128)]
        last = tail_chain(xb0, 0, cols, tall.at[0])
        mk = jnp.concatenate([m_v[...] > 0] * gpi, axis=1)
        lb = jnp.concatenate([last.astype(_BF)] * gpi, axis=1)
        parts = []
        for r in range(0, D, 128):
            parts.append(jnp.where(mk, lb, xin[r:r + 16]))
            parts.append(xin[r + 16:min(r + 128, D)])
        xt = jnp.concatenate(parts, axis=0).T
        for q in range(gpi):
            x_v[jc * gpi + q] = _u32(xt[128 * q:128 * q + 128])
            xu_v[jc * gpi + q] = _u32(_half(xt[128 * q:128 * q + 128]))
        xtl = jnp.concatenate([x_v[jc * gpi + q, 48:64, _KM:] for q in range(gpi)], axis=0)
        build_xb(_bf(xtl).astype(_F32), gpi, xb, jc * gpi)

        @pl.when(j + 1 < nl)
        def _():
            for c in loop_cps(j + 1):
                c.wait()

        return jnp.minimum(jc + 1, nl - 1)

    for c in loop_cps(0):
        c.wait()
    lax.fori_loop(0, nl, ploop, jnp.int32(0))
    pltpu.make_async_copy(o_v.at[:, 0:t0], o_hbm.at[:, 0:t0], sem.at[0]).start()

    def mloop(i, gn):
        r0 = pl.multiple_of(i * ts, 128)
        t_in, t_out, t_e = tall.at[i], tall.at[i + 1], te_v.at[i]

        def proj(ref, k, base, nn, ca, cb):
            xs = (ref[2 * i], ref[2 * i + 1])
            c2 = min(max(nn * 128, ca), cb)
            inits = []
            for lo, hi, two in ((ca, c2, True), (c2, cb, False)):
                if lo >= hi:
                    continue
                segs = [(0, _EA)] + ([] if two else [(96, 112)])
                na = sum(b - a for a, b in segs)
                ta = _dot(_bf(_cat([x[a // 2:b // 2, _KM:] for x in xs for a, b in segs], 0)), rdm(k, lo, hi, _KM, D))
                cs = slice(base + lo, base + hi)
                parts = []
                for q in range(2):
                    parts.append(ta[q * na:q * na + _EA])
                    parts.append(t_e[q * ne:(q + 1) * ne, cs])
                    if two:
                        parts.append(t_in[32 * q:32 * q + 32, cs])
                    else:
                        parts.append(ta[q * na + _EA:(q + 1) * na])
                        parts.append(t_in[32 * q + 16:32 * q + 32, cs])
                inits.append(jnp.concatenate(parts, axis=0))
            xm = _bf(jnp.concatenate([x[:, 0:_KM] for x in xs], axis=0))
            return _dot(xm, rdm(k, ca, cb, 0, _KM)) + _cat(inits, 1)

        hs = [[], []]
        for ca in range(0, F, _GC * 128):
            cb = min(ca + _GC * 128, F)
            g = proj(x_v, 'g', 0, _N2[0], ca, cb)
            u = proj(xu_v, 'u', F, _N2[1], ca, cb)
            for q in range(2):
                hs[q].append(_act(g[q * 128:(q + 1) * 128], u[q * 128:(q + 1) * 128]))
        for q in range(2):
            h = _cat(hs[q], 1)
            oq = pl.ds(pl.multiple_of(t0 + r0 + q * 128, 128), 128)
            cuts = _DSPLIT if q == 1 else (0, D)
            for a, b in zip(cuts[:-1], cuts[1:]):
                o_v[a:b, oq] = _dot_nt(rdm('d', 0, F, a, b), h).astype(_BF)
                pltpu.make_async_copy(o_v.at[a:b, oq], o_hbm.at[a:b, oq], sem.at[0]).start()
        cols = [(wt_v.at[c // lf], b * lf + c % lf, b * F + c, (0, 16) if c < nn * 128 else (16,))
                for b, nn in enumerate(_N2) for c in range(0, F, 128)]
        tail_chain(xb, gn, cols, t_out, None, _TREE)
        return jnp.minimum(gn + 2, 2 * (nm - 1))

    lax.fori_loop(0, nm, mloop, jnp.int32(2))
    keep = pltpu.make_async_copy(tall.at[1, 16:24, 0:128], keep_hbm, sem.at[1])
    keep.start()
    pltpu.make_async_copy(o_v, o_hbm, sem.at[0]).wait()
    keep.wait()


@jax.jit
def pallas_standalone__geglu_ffn__prompt_kernel(x, w_gate, w_up, w_down):
    B, S, D = x.shape
    F = w_gate.shape[1]
    M = B * S
    lf = F // _NL
    ng = (M - _T0) // 128
    ne = 96 - _EA
    assert D == _KM + _KT and F % (128 * _NL) == 0 and (M - _T0) % _TS == 0 and ng % _NL == 0
    assert 3 * lf + (M - _T0) // _NL <= _SLOTW and M <= _SLOTW and _KT * (1 + 2 * _NL) <= D
    xT = x.reshape(M, D).T
    wdT = w_down.T
    outT, _ = pl.pallas_call(
        _kernel,
        in_specs=[pl.BlockSpec(memory_space=pl.ANY)] * 4,
        out_specs=[pl.BlockSpec(memory_space=pl.ANY)] * 2,
        out_shape=[jax.ShapeDtypeStruct((D, M), x.dtype), jax.ShapeDtypeStruct((8, 128), _F32)],
        scratch_shapes=[
            pltpu.VMEM((_NL + 1, D, _SLOTW), _BF),
            pltpu.VMEM((_NL, D // 2, lf), _U32),
            pltpu.VMEM((_NL, D // 2, lf), _U32),
            pltpu.VMEM((_NL, D // 2, lf), _U32),
            pltpu.VMEM((_T0 // 2, D), _U32), pltpu.VMEM((_T0 // 2, D), _U32),
            pltpu.VMEM((ng, 64, D), _U32), pltpu.VMEM((ng, 64, D), _U32),
            pltpu.VMEM((3, ng * ne, _KT), _BF),
            pltpu.VMEM((D, _T0), _F32),
            pltpu.VMEM((D, M), _BF),
            pltpu.VMEM((_NL, _KT, 4096), _F32),
            pltpu.VMEM((ng, _KT, 32, 128), _F32),
            pltpu.VMEM((2, _KT, 32, 128), _F32),
            pltpu.VMEM(((M - _T0) // _TS + 1, 64, 2 * F), _F32),
            pltpu.VMEM(((M - _T0) // _TS, 2 * ne, 2 * F), _F32),
            pltpu.VMEM((16, 128), _F32),
            pltpu.SemaphoreType.DMA((3 + _NL,)),
        ],
        compiler_params=pltpu.CompilerParams(
            vmem_limit_bytes=112 * 1024 * 1024,
            disable_bounds_checks=True,
            disable_semaphore_checks=True,
        ),
    )(xT, w_gate, w_up, wdT)
    return outT.T.reshape(B, S, D)
```

```python
import jax
import jax.numpy as jnp
from jax import lax
import jax.experimental.pallas as pl
import jax.experimental.pallas.tpu as pltpu

_NT = (((1,), (1,)), ((), ()))
_F32 = jnp.float32
_BF = jnp.bfloat16
_U32 = jnp.uint32
_C0 = 0.7978845608028654
_C1 = _C0 * 0.044715

_KM = 512
_KT = 64
_KG = 8
_T0 = 512
_TS = 256
_NL = 4
_SLOTW = 3840
_EA = 48
_NF1 = 10
_GC = 4
_DSPLIT = (0, 448, 576)
_SW = (4, (1, 3, 116))
_PSW = (3, (0, 0, 0))


def _act(g, uh):
    t = jnp.tanh(g * (_C0 + _C1 * (g * g)))
    return ((g * (1.0 + t)) * uh).astype(_BF)


def _half(x):
    return (x.astype(_F32) * 0.5).astype(_BF)


def _mo(v):
    return v if isinstance(v, int) else pl.multiple_of(v, 128)


def _dot(a, b):
    return jnp.dot(a, b, preferred_element_type=_F32)


def _dot_nt(a, b):
    return lax.dot_general(a, b, _NT, preferred_element_type=_F32)


def _cat(parts, axis):
    return parts[0] if len(parts) == 1 else jnp.concatenate(parts, axis=axis)


def _bf(x):
    return pltpu.bitcast(x, _BF)


def _u32(x):
    return pltpu.bitcast(x, _U32)


def _kernel(xT_hbm, wg_hbm, wu_hbm, wd_hbm, o_hbm, keep_hbm,
            buf, pg, pu, pd, x0_v, xu0_v, x_v, xu_v, xe_v, acc_v, o_v, wt_v, xb, xb0, tall, te_v, m_v, sem):
    D, M = o_v.shape
    F = wg_hbm.shape[1]
    t0, ts, nl = _T0, _TS, _NL
    lf = F // nl
    nm = (M - t0) // ts
    xr = (M - t0) // nl
    gpi = xr // 128
    ng = (M - t0) // 128
    ne = 96 - _EA
    f1 = _NF1 * 128
    hbm = dict(x=xT_hbm, g=wg_hbm, u=wu_hbm, d=wd_hbm)
    posl = dict(g=0, u=lf, d=2 * lf, x=3 * lf)
    XT = t0
    packed = dict(g=pg, u=pu, d=pd)

    def cp(k, r0, r1, off, size, slot, dr0, pos, s):
        return pltpu.make_async_copy(hbm[k].at[r0:r1, pl.ds(_mo(off), size)],
                                     buf.at[slot, dr0:dr0 + r1 - r0, pos:pos + size], sem.at[s])

    def band(k, j):
        return _KT * (1 + 2 * j + (k == 'u'))

    def tail_cps(c0, c1, s):
        cps = []
        for j in range(nl):
            a, b = max(c0, j * lf), min(c1, (j + 1) * lf)
            if a < b:
                cps += [cp(k, _KM, D, a, b - a, 0, band(k, j), XT + a - j * lf, s) for k in 'gu']
        return cps

    f1_cps = [cp('x', _KM, D, t0, M - t0, 0, 0, XT, 1)] + tail_cps(0, f1, 1)
    f2_cps = [cp('x', 0, D, 0, t0, 0, 0, 0, 2)] + tail_cps(f1, F, 2)

    def loop_cps(j):
        s, slot = 3 + j, 1 + j
        return ([cp(k, 0, _KM, j * lf, lf, slot, 0, posl[k], s) for k in 'gu']
                + [cp('d', 0, D, j * lf, lf, slot, 0, posl['d'], s),
                   cp('x', 0, D, t0 + j * xr, xr, slot, 0, posl['x'], s)])

    def fresh(k, j, rows):
        w = buf[1 + j, 0:rows, posl[k]:posl[k] + lf]
        packed[k][j, 0:rows // 2, 0:lf] = _u32(w)
        return w

    def rdm(k, c0, c1, r0=0, r1=D):
        parts = []
        for s in range(nl):
            a, b = max(c0, s * lf), min(c1, (s + 1) * lf)
            if a < b:
                parts.append(packed[k][s, r0 // 2:r1 // 2, a - s * lf:b - s * lf])
        return _bf(_cat(parts, 1))

    for c in f1_cps + f2_cps + [c_ for j in range(nl) for c_ in loop_cps(j)]:
        c.start()

    acc_v[...] = jnp.zeros_like(acc_v)
    m_v[...] = jnp.zeros_like(m_v)

    def build_xb(xtl, ngrp, dst, g0):
        never = m_v[0:8, :] > 0
        zero = jnp.zeros((8, 128), _F32)
        prev = None
        for k in range(_KT):
            col = jnp.broadcast_to(xtl[:, k:k + 1], (32 * ngrp, 128))
            for q in range(ngrp):
                for r in range(0, 32, 8):
                    v = col[32 * q + r:32 * q + r + 8]
                    prev = v if prev is None else v + lax.select(never, prev, zero)
                    dst[g0 + q, k, r:r + 8, :] = prev

    def tail_chain(xsrc, g0, cols, dst, sw):
        never = m_v[...] > 0
        xq = [xsrc.at[g0 + q] for q in range(2)]
        ncol, sched = sw
        left = 4 * len(cols)
        prev = None
        for c0 in range(0, len(cols), ncol):
            grp = cols[c0:c0 + ncol]
            wk = {}
            for q in range(2):
                for rr in (0, 16):
                    npair = sched[1] if left <= sched[2] else sched[0]
                    left -= len(grp)
                    accs = [None] * len(grp)
                    for k0 in range(0, _KT, _KG):
                        x8 = xq[q][k0:k0 + _KG, rr:rr + 16, :]
                        for ci, (wref, wc, _) in enumerate(grp):
                            if (ci, k0) not in wk:
                                wk[(ci, k0)] = jnp.concatenate(
                                    [lax.broadcast_in_dim(wref[k:k + 1, wc:wc + 128], (1, 16, 128), (1, 2))
                                     for k in range(k0, k0 + _KG)], axis=0)
                            p = x8 * wk[(ci, k0)]
                            head, lo = (p[0], 1) if accs[ci] is None else (accs[ci], 0)
                            if prev is not None:
                                head = lax.select(never, prev, head)
                            terms = [head[None]]
                            if npair:
                                terms.append(p[lo:lo + npair] + p[lo + npair:lo + 2 * npair])
                                lo += 2 * npair
                            terms.append(p[lo:])
                            accs[ci] = prev = jnp.sum(_cat(terms, 0), axis=0)
                    for ci, (_, _, col) in enumerate(grp):
                        dst[32 * q + rr:32 * q + rr + 16, pl.ds(_mo(col), 128)] = accs[ci]
        return prev

    def filler(lhs, c0, c1):
        for j in range(nl):
            ca, cb = max(c0, j * lf) - j * lf, min(c1, (j + 1) * lf) - j * lf
            if ca >= cb:
                continue
            for b, k in enumerate('gu'):
                wp = _u32(buf[0, band(k, j):band(k, j) + _KT, XT + ca:XT + cb])
                packed[k][j, _KM // 2:D // 2, ca:cb] = wp
                w = _bf(wp)
                te = _dot(lhs[b], w)
                gc0 = b * F + j * lf
                for t in range(nm):
                    te_v[t, :, gc0 + ca:gc0 + cb] = te[2 * ne * t:2 * ne * (t + 1)]
                wt_v[j, :, b * lf + ca:b * lf + cb] = w.astype(_F32) * 0.5 if b else w.astype(_F32)

    for c in f1_cps:
        c.wait()
    xt = buf[0, 0:_KT, XT:XT + M - t0].T
    xe = jnp.concatenate([xt[128 * q + _EA:128 * q + 96] for q in range(ng)], axis=0)
    lhs = (xe, _half(xe))
    xe_v[0] = lhs[0]
    xe_v[1] = lhs[1]
    xe_v[2, 0:64, :] = jnp.concatenate([xt[96:128], xt[224:256]], axis=0)
    filler(lhs, 0, f1)

    for c in f2_cps:
        c.wait()
    filler((xe_v[0], xe_v[1]), f1, F)
    x0t = buf[0, :, 0:t0].T
    x0_v[...] = _u32(x0t)
    xu0_v[...] = _u32(_half(x0t))
    build_xb(xe_v[2, 0:64, :].astype(_F32), 2, xb0, 0)

    def ploop(j, jc):
        def wfull(k):
            return jnp.concatenate([fresh(k, j, _KM), _bf(packed[k][j, _KM // 2:D // 2, 0:lf])], axis=0)

        g = _dot(_bf(x0_v[...]), wfull('g'))
        u = _dot(_bf(xu0_v[...]), wfull('u'))
        a = acc_v[...] + _dot_nt(fresh('d', j, D), _act(g, u))
        acc_v[...] = a
        o_v[:, 0:t0] = a.astype(_BF)
        xin = buf[1 + jc, :, posl['x']:posl['x'] + xr]
        wq = wt_v.at[jc]
        cols = [(wq, b * lf + c, b * F + jc * lf + c) for b in range(2) for c in range(0, lf, 128)]
        last = tail_chain(xb0, 0, cols, tall.at[0], _PSW)
        mk = jnp.concatenate([m_v[...] > 0] * gpi, axis=1)
        lb = jnp.concatenate([last.astype(_BF)] * gpi, axis=1)
        parts = []
        for r in range(0, D, 128):
            parts.append(jnp.where(mk, lb, xin[r:r + 16]))
            parts.append(xin[r + 16:min(r + 128, D)])
        xt = jnp.concatenate(parts, axis=0).T
        for q in range(gpi):
            x_v[jc * gpi + q] = _u32(xt[128 * q:128 * q + 128])
            xu_v[jc * gpi + q] = _u32(_half(xt[128 * q:128 * q + 128]))
        xtl = jnp.concatenate([x_v[jc * gpi + q, 48:64, _KM:] for q in range(gpi)], axis=0)
        build_xb(_bf(xtl).astype(_F32), gpi, xb, jc * gpi)

        @pl.when(j + 1 < nl)
        def _():
            for c in loop_cps(j + 1):
                c.wait()

        return jnp.minimum(jc + 1, nl - 1)

    for c in loop_cps(0):
        c.wait()
    lax.fori_loop(0, nl, ploop, jnp.int32(0))
    pltpu.make_async_copy(o_v.at[:, 0:t0], o_hbm.at[:, 0:t0], sem.at[0]).start()

    def mloop(i, gn):
        r0 = pl.multiple_of(i * ts, 128)
        t_in, t_out, t_e = tall.at[i], tall.at[i + 1], te_v.at[i]

        def proj(ref, k, base, ca, cb):
            xs = (ref[2 * i], ref[2 * i + 1])
            ta = _dot(_bf(jnp.concatenate([x[0:_EA // 2, _KM:] for x in xs], axis=0)), rdm(k, ca, cb, _KM, D))
            cs = slice(base + ca, base + cb)
            parts = []
            for q in range(2):
                parts += [ta[q * _EA:(q + 1) * _EA], t_e[q * ne:(q + 1) * ne, cs], t_in[32 * q:32 * q + 32, cs]]
            init = jnp.concatenate(parts, axis=0)
            xm = _bf(jnp.concatenate([x[:, 0:_KM] for x in xs], axis=0))
            return _dot(xm, rdm(k, ca, cb, 0, _KM)) + init

        hs = [[], []]
        for ca in range(0, F, _GC * 128):
            cb = min(ca + _GC * 128, F)
            g = proj(x_v, 'g', 0, ca, cb)
            u = proj(xu_v, 'u', F, ca, cb)
            for q in range(2):
                hs[q].append(_act(g[q * 128:(q + 1) * 128], u[q * 128:(q + 1) * 128]))
        for q in range(2):
            h = _cat(hs[q], 1)
            oq = pl.ds(pl.multiple_of(t0 + r0 + q * 128, 128), 128)
            cuts = _DSPLIT if q == 1 else (0, D)
            for a, b in zip(cuts[:-1], cuts[1:]):
                o_v[a:b, oq] = _dot_nt(rdm('d', 0, F, a, b), h).astype(_BF)
                pltpu.make_async_copy(o_v.at[a:b, oq], o_hbm.at[a:b, oq], sem.at[0]).start()
        cols = [(wt_v.at[c // lf], b * lf + c % lf, b * F + c) for b in range(2) for c in range(0, F, 128)]
        tail_chain(xb, gn, cols, t_out, _SW)
        return jnp.minimum(gn + 2, 2 * (nm - 1))

    lax.fori_loop(0, nm, mloop, jnp.int32(2))
    keep = pltpu.make_async_copy(tall.at[1, 16:24, 0:128], keep_hbm, sem.at[1])
    keep.start()
    pltpu.make_async_copy(o_v, o_hbm, sem.at[0]).wait()
    keep.wait()


@jax.jit
def pallas_standalone__geglu_ffn__prompt_kernel(x, w_gate, w_up, w_down):
    B, S, D = x.shape
    F = w_gate.shape[1]
    M = B * S
    lf = F // _NL
    ng = (M - _T0) // 128
    ne = 96 - _EA
    assert D == _KM + _KT and F % (128 * _NL) == 0 and (M - _T0) % _TS == 0 and ng % _NL == 0
    assert 3 * lf + (M - _T0) // _NL <= _SLOTW and M <= _SLOTW and _KT * (1 + 2 * _NL) <= D
    xT = x.reshape(M, D).T
    wdT = w_down.T
    outT, _ = pl.pallas_call(
        _kernel,
        in_specs=[pl.BlockSpec(memory_space=pl.ANY)] * 4,
        out_specs=[pl.BlockSpec(memory_space=pl.ANY)] * 2,
        out_shape=[jax.ShapeDtypeStruct((D, M), x.dtype), jax.ShapeDtypeStruct((8, 128), _F32)],
        scratch_shapes=[
            pltpu.VMEM((_NL + 1, D, _SLOTW), _BF),
            pltpu.VMEM((_NL, D // 2, lf), _U32),
            pltpu.VMEM((_NL, D // 2, lf), _U32),
            pltpu.VMEM((_NL, D // 2, lf), _U32),
            pltpu.VMEM((_T0 // 2, D), _U32),
            pltpu.VMEM((_T0 // 2, D), _U32),
            pltpu.VMEM((ng, 64, D), _U32),
            pltpu.VMEM((ng, 64, D), _U32),
            pltpu.VMEM((3, ng * ne, _KT), _BF),
            pltpu.VMEM((D, _T0), _F32),
            pltpu.VMEM((D, M), _BF),
            pltpu.VMEM((_NL, _KT, 4096), _F32),
            pltpu.VMEM((ng, _KT, 32, 128), _F32),
            pltpu.VMEM((2, _KT, 32, 128), _F32),
            pltpu.VMEM(((M - _T0) // _TS + 1, 64, 2 * F), _F32),
            pltpu.VMEM(((M - _T0) // _TS, 2 * ne, 2 * F), _F32),
            pltpu.VMEM((16, 128), _F32),
            pltpu.SemaphoreType.DMA((3 + _NL,)),
        ],
        compiler_params=pltpu.CompilerParams(
            vmem_limit_bytes=112 * 1024 * 1024,
            disable_bounds_checks=True,
            disable_semaphore_checks=True,
        ),
    )(xT, w_gate, w_up, wdT)
    return outT.T.reshape(B, S, D)
```

```python
import jax
import jax.numpy as jnp
from jax import lax
import jax.experimental.pallas as pl
import jax.experimental.pallas.tpu as pltpu

_NT = (((1,), (1,)), ((), ()))
_F32 = jnp.float32
_BF = jnp.bfloat16
_U32 = jnp.uint32
_C0 = 0.7978845608028654
_C1 = _C0 * 0.044715

_KM = 512
_KT = 64
_KG = 8
_T0 = 512
_TS = 256
_NL = 4
_SLOTW = 3840
_EA = 48
_NF1 = 10
_GC = 4
_DSPLIT = (0, 448, 576)
_SW = (4, (1, 3, 116))
_PSW = (3, (0, 0, 0))


def _act(g, uh):
    t = jnp.tanh(g * (_C0 + _C1 * (g * g)))
    return ((g * (1.0 + t)) * uh).astype(_BF)


def _half(x):
    return (x.astype(_F32) * 0.5).astype(_BF)


def _mo(v):
    return v if isinstance(v, int) else pl.multiple_of(v, 128)


def _dot(a, b):
    return jnp.dot(a, b, preferred_element_type=_F32)


def _dot_nt(a, b):
    return lax.dot_general(a, b, _NT, preferred_element_type=_F32)


def _cat(parts, axis):
    return parts[0] if len(parts) == 1 else jnp.concatenate(parts, axis=axis)


def _bf(x):
    return pltpu.bitcast(x, _BF)


def _u32(x):
    return pltpu.bitcast(x, _U32)


def _kernel(xT_hbm, wg_hbm, wu_hbm, wd_hbm, o_hbm, keep_hbm,
            buf, pg, pu, pd, x0_v, xu0_v, x_v, xu_v, xe_v, acc_v, o_v, wt_v, xb, xb0, tall, te_v, m_v, sem):
    D, M = o_v.shape
    F = wg_hbm.shape[1]
    t0, ts, nl = _T0, _TS, _NL
    lf = F // nl
    nm = (M - t0) // ts
    xr = (M - t0) // nl
    gpi = xr // 128
    ng = (M - t0) // 128
    ne = 96 - _EA
    f1 = _NF1 * 128
    hbm = dict(x=xT_hbm, g=wg_hbm, u=wu_hbm, d=wd_hbm)
    posl = dict(g=0, u=lf, d=2 * lf, x=3 * lf)
    XT = t0
    packed = dict(g=pg, u=pu, d=pd)

    def cp(k, r0, r1, off, size, slot, dr0, pos, s):
        return pltpu.make_async_copy(hbm[k].at[r0:r1, pl.ds(_mo(off), size)],
                                     buf.at[slot, dr0:dr0 + r1 - r0, pos:pos + size], sem.at[s])

    def band(k, j):
        return _KT * (1 + 2 * j + (k == 'u'))

    def tail_cps(c0, c1, s):
        cps = []
        for j in range(nl):
            a, b = max(c0, j * lf), min(c1, (j + 1) * lf)
            if a < b:
                cps += [cp(k, _KM, D, a, b - a, 0, band(k, j), XT + a - j * lf, s) for k in 'gu']
        return cps

    f1_cps = [cp('x', _KM, D, t0, M - t0, 0, 0, XT, 1)] + tail_cps(0, f1, 1)
    f2_cps = [cp('x', 0, D, 0, t0, 0, 0, 0, 2)] + tail_cps(f1, F, 2)

    def loop_cps(j):
        s, slot = 3 + j, 1 + j
        return ([cp(k, 0, _KM, j * lf, lf, slot, 0, posl[k], s) for k in 'gu']
                + [cp('d', 0, D, j * lf, lf, slot, 0, posl['d'], s),
                   cp('x', 0, D, t0 + j * xr, xr, slot, 0, posl['x'], s)])

    def fresh(k, j, rows):
        w = buf[1 + j, 0:rows, posl[k]:posl[k] + lf]
        packed[k][j, 0:rows // 2, 0:lf] = _u32(w)
        return w

    def rdm(k, c0, c1, r0=0, r1=D):
        parts = []
        for s in range(nl):
            a, b = max(c0, s * lf), min(c1, (s + 1) * lf)
            if a < b:
                parts.append(packed[k][s, r0 // 2:r1 // 2, a - s * lf:b - s * lf])
        return _bf(_cat(parts, 1))

    for c in f1_cps + f2_cps + [c_ for j in range(nl) for c_ in loop_cps(j)]:
        c.start()

    acc_v[...] = jnp.zeros_like(acc_v)
    m_v[...] = jnp.zeros_like(m_v)

    def build_xb(xtl, ngrp, dst, g0):
        never = m_v[0:8, :] > 0
        zero = jnp.zeros((8, 128), _F32)
        prev = None
        for k in range(_KT):
            col = jnp.broadcast_to(xtl[:, k:k + 1], (32 * ngrp, 128))
            for q in range(ngrp):
                for r in range(0, 32, 8):
                    v = col[32 * q + r:32 * q + r + 8]
                    prev = v if prev is None else v + lax.select(never, prev, zero)
                    dst[g0 + q, k, r:r + 8, :] = prev

    def tail_chain(xsrc, g0, cols, dst, sw):
        never = m_v[...] > 0
        xq = [xsrc.at[g0 + q] for q in range(2)]
        ncol, sched = sw
        left = 4 * len(cols)
        prev = None
        for c0 in range(0, len(cols), ncol):
            grp = cols[c0:c0 + ncol]
            wk = {}
            for q in range(2):
                for rr in (0, 16):
                    npair = sched[1] if left <= sched[2] else sched[0]
                    left -= len(grp)
                    accs = [None] * len(grp)
                    for k0 in range(0, _KT, _KG):
                        x8 = xq[q][k0:k0 + _KG, rr:rr + 16, :]
                        for ci, (wref, wc, _) in enumerate(grp):
                            if (ci, k0) not in wk:
                                wk[(ci, k0)] = jnp.concatenate(
                                    [lax.broadcast_in_dim(wref[k:k + 1, wc:wc + 128], (1, 16, 128), (1, 2))
                                     for k in range(k0, k0 + _KG)], axis=0)
                            p = x8 * wk[(ci, k0)]
                            head, lo = (p[0], 1) if accs[ci] is None else (accs[ci], 0)
                            if prev is not None:
                                head = lax.select(never, prev, head)
                            terms = [head[None]]
                            if npair:
                                terms.append(p[lo:lo + npair] + p[lo + npair:lo + 2 * npair])
                                lo += 2 * npair
                            terms.append(p[lo:])
                            accs[ci] = prev = jnp.sum(_cat(terms, 0), axis=0)
                    for ci, (_, _, col) in enumerate(grp):
                        dst[32 * q + rr:32 * q + rr + 16, pl.ds(_mo(col), 128)] = accs[ci]
        return prev

    def filler(lhs, c0, c1):
        for j in range(nl):
            ca, cb = max(c0, j * lf) - j * lf, min(c1, (j + 1) * lf) - j * lf
            if ca >= cb:
                continue
            for b, k in enumerate('gu'):
                wp = _u32(buf[0, band(k, j):band(k, j) + _KT, XT + ca:XT + cb])
                packed[k][j, _KM // 2:D // 2, ca:cb] = wp
                w = _bf(wp)
                te = _dot(lhs[b], w)
                gc0 = b * F + j * lf
                for t in range(nm):
                    te_v[t, :, gc0 + ca:gc0 + cb] = te[2 * ne * t:2 * ne * (t + 1)]
                wt_v[j, :, b * lf + ca:b * lf + cb] = w.astype(_F32) * 0.5 if b else w.astype(_F32)

    for c in f1_cps:
        c.wait()
    xt = buf[0, 0:_KT, XT:XT + M - t0].T
    xe = jnp.concatenate([xt[128 * q + _EA:128 * q + 96] for q in range(ng)], axis=0)
    lhs = (xe, _half(xe))
    xe_v[0] = lhs[0]
    xe_v[1] = lhs[1]
    xe_v[2, 0:64, :] = jnp.concatenate([xt[96:128], xt[224:256]], axis=0)
    filler(lhs, 0, f1)

    for c in f2_cps:
        c.wait()
    filler((xe_v[0], xe_v[1]), f1, F)
    x0t = buf[0, :, 0:t0].T
    x0_v[...] = _u32(x0t)
    xu0_v[...] = _u32(_half(x0t))
    build_xb(xe_v[2, 0:64, :].astype(_F32), 2, xb0, 0)

    def ploop(j, jc):
        def wfull(k):
            return jnp.concatenate([fresh(k, j, _KM), _bf(packed[k][j, _KM // 2:D // 2, 0:lf])], axis=0)

        g = _dot(_bf(x0_v[...]), wfull('g'))
        u = _dot(_bf(xu0_v[...]), wfull('u'))
        a = acc_v[...] + _dot_nt(fresh('d', j, D), _act(g, u))
        acc_v[...] = a
        o_v[:, 0:t0] = a.astype(_BF)
        xin = buf[1 + jc, :, posl['x']:posl['x'] + xr]
        wq = wt_v.at[jc]
        cols = [(wq, b * lf + c, b * F + jc * lf + c) for b in range(2) for c in range(0, lf, 128)]
        last = tail_chain(xb0, 0, cols, tall.at[0], _PSW)
        mk = jnp.concatenate([m_v[...] > 0] * gpi, axis=1)
        lb = jnp.concatenate([last.astype(_BF)] * gpi, axis=1)
        parts = []
        for r in range(0, D, 128):
            parts.append(jnp.where(mk, lb, xin[r:r + 16]))
            parts.append(xin[r + 16:min(r + 128, D)])
        xt = jnp.concatenate(parts, axis=0).T
        for q in range(gpi):
            x_v[jc * gpi + q] = _u32(xt[128 * q:128 * q + 128])
            xu_v[jc * gpi + q] = _u32(_half(xt[128 * q:128 * q + 128]))
        xtl = jnp.concatenate([x_v[jc * gpi + q, 48:64, _KM:] for q in range(gpi)], axis=0)
        build_xb(_bf(xtl).astype(_F32), gpi, xb, jc * gpi)

        @pl.when(j + 1 < nl)
        def _():
            for c in loop_cps(j + 1):
                c.wait()

        return jnp.minimum(jc + 1, nl - 1)

    for c in loop_cps(0):
        c.wait()
    lax.fori_loop(0, nl, ploop, jnp.int32(0))
    pltpu.make_async_copy(o_v.at[:, 0:t0], o_hbm.at[:, 0:t0], sem.at[0]).start()

    def mloop(i, gn):
        r0 = pl.multiple_of(i * ts, 128)
        t_in, t_out, t_e = tall.at[i], tall.at[i + 1], te_v.at[i]

        def proj(ref, k, base, ca, cb):
            xs = (ref[2 * i], ref[2 * i + 1])
            ta = _dot(_bf(jnp.concatenate([x[0:_EA // 2, _KM:] for x in xs], axis=0)), rdm(k, ca, cb, _KM, D))
            cs = slice(base + ca, base + cb)
            parts = []
            for q in range(2):
                parts += [ta[q * _EA:(q + 1) * _EA], t_e[q * ne:(q + 1) * ne, cs], t_in[32 * q:32 * q + 32, cs]]
            init = jnp.concatenate(parts, axis=0)
            xm = _bf(jnp.concatenate([x[:, 0:_KM] for x in xs], axis=0))
            return _dot(xm, rdm(k, ca, cb, 0, _KM)) + init

        hs = [[], []]
        for ca in range(0, F, _GC * 128):
            cb = min(ca + _GC * 128, F)
            g = proj(x_v, 'g', 0, ca, cb)
            u = proj(xu_v, 'u', F, ca, cb)
            for q in range(2):
                hs[q].append(_act(g[q * 128:(q + 1) * 128], u[q * 128:(q + 1) * 128]))
        for q in range(2):
            h = _cat(hs[q], 1)
            oq = pl.ds(pl.multiple_of(t0 + r0 + q * 128, 128), 128)
            cuts = _DSPLIT if q == 1 else (0, D)
            for a, b in zip(cuts[:-1], cuts[1:]):
                o_v[a:b, oq] = _dot_nt(rdm('d', 0, F, a, b), h).astype(_BF)
                pltpu.make_async_copy(o_v.at[a:b, oq], o_hbm.at[a:b, oq], sem.at[0]).start()
        cols = [(wt_v.at[c // lf], b * lf + c % lf, b * F + c) for b in range(2) for c in range(0, F, 128)]
        tail_chain(xb, gn, cols, t_out, _SW)
        return jnp.minimum(gn + 2, 2 * (nm - 1))

    lax.fori_loop(0, nm, mloop, jnp.int32(2))
    keep = pltpu.make_async_copy(tall.at[1, 16:24, 0:128], keep_hbm, sem.at[1])
    keep.start()
    pltpu.make_async_copy(o_v, o_hbm, sem.at[0]).wait()
    keep.wait()


@jax.jit
def pallas_standalone__geglu_ffn__prompt_kernel(x, w_gate, w_up, w_down):
    B, S, D = x.shape
    F = w_gate.shape[1]
    M = B * S
    lf = F // _NL
    ng = (M - _T0) // 128
    ne = 96 - _EA
    assert D == _KM + _KT and F % (128 * _NL) == 0 and (M - _T0) % _TS == 0 and ng % _NL == 0
    assert 3 * lf + (M - _T0) // _NL <= _SLOTW and M <= _SLOTW and _KT * (1 + 2 * _NL) <= D
    nochecks = {k: True for k in ('disable_bounds_checks', 'disable_semaphore_checks')
                if hasattr(pltpu.CompilerParams, k)}
    xT = x.reshape(M, D).T
    wdT = w_down.T
    outT, _ = pl.pallas_call(
        _kernel,
        in_specs=[pl.BlockSpec(memory_space=pl.ANY)] * 4,
        out_specs=[pl.BlockSpec(memory_space=pl.ANY)] * 2,
        out_shape=[jax.ShapeDtypeStruct((D, M), x.dtype), jax.ShapeDtypeStruct((8, 128), _F32)],
        scratch_shapes=[
            pltpu.VMEM((_NL + 1, D, _SLOTW), _BF),
            pltpu.VMEM((_NL, D // 2, lf), _U32),
            pltpu.VMEM((_NL, D // 2, lf), _U32),
            pltpu.VMEM((_NL, D // 2, lf), _U32),
            pltpu.VMEM((_T0 // 2, D), _U32),
            pltpu.VMEM((_T0 // 2, D), _U32),
            pltpu.VMEM((ng, 64, D), _U32),
            pltpu.VMEM((ng, 64, D), _U32),
            pltpu.VMEM((3, ng * ne, _KT), _BF),
            pltpu.VMEM((D, _T0), _F32),
            pltpu.VMEM((D, M), _BF),
            pltpu.VMEM((_NL, _KT, 4096), _F32),
            pltpu.VMEM((ng, _KT, 32, 128), _F32),
            pltpu.VMEM((2, _KT, 32, 128), _F32),
            pltpu.VMEM(((M - _T0) // _TS + 1, 64, 2 * F), _F32),
            pltpu.VMEM(((M - _T0) // _TS, 2 * ne, 2 * F), _F32),
            pltpu.VMEM((16, 128), _F32),
            pltpu.SemaphoreType.DMA((3 + _NL,)),
        ],
        compiler_params=pltpu.CompilerParams(vmem_limit_bytes=112 * 1024 * 1024, **nochecks),
    )(xT, w_gate, w_up, wdT)
    return outT.T.reshape(B, S, D)
```
